```python
import jax
import jax.numpy as jnp

def _softmax(x, axis=-1):
    return jax.nn.softmax(x, axis=axis)
def _gelu(x):
    return jax.nn.gelu(x, approximate=True)
def _silu(x):
    return jax.nn.silu(x)
def _sigmoid(x):
    return jax.nn.sigmoid(x)
def _layernorm(x, axis=-1, eps=1e-5):
    m = jnp.mean(x, axis=axis, keepdims=True)
    v = jnp.var(x, axis=axis, keepdims=True)
    return (x - m) / jnp.sqrt(v + eps)
def _scatter_add(tgt, idx, src, axis=0):
    return tgt.at[idx].add(src)
def _segment_sum(src, seg, n):
    return jax.ops.segment_sum(src, seg, n)
class _Rng:
    def __init__(self, key):
        self._k = key
    def _next(self):
        self._k, sub = jax.random.split(self._k)
        return sub
    def normal(self, shape):
        return jax.random.normal(self._next(), shape, dtype=jnp.bfloat16)
    def randint(self, lo, hi, shape):
        return jax.random.randint(self._next(), shape, lo, hi, dtype=jnp.int32)
    def uniform(self, shape, lo=0.0, hi=1.0):
        return jax.random.uniform(self._next(), shape, jnp.bfloat16, lo, hi)
    def permutation(self, n):
        return jax.random.permutation(self._next(), n)


kernel_name = 'interleave_layers__linear_attn_block__mixer_channel_mlp__prompt'

def _fwd_setup_inputs():
    _rng = _Rng(jax.random.key(int.from_bytes(__import__("os").urandom(4), "little")))
    _w = (lambda a: (lambda t: t.astype(jnp.bfloat16) if jnp.issubdtype(t.dtype, jnp.floating) else t)(jnp.asarray(a)))
    def _A_setup():
        B, S, D = 1, 2048, 576
        return {
            "x": _w((lambda *s: _rng.normal(s) * 0.05)(B, S, D)),
            "wqkv": _w((lambda *s: _rng.normal(s) * 0.05)(D, 3 * D)),
            "wo": _w((lambda *s: _rng.normal(s) * 0.05)(D, D)),
        }
    _A_in = _A_setup()

    def _B_setup():
        B, S, D, F = 1, 2048, 576, 4608
        return {
            "x": _w((lambda *s: _rng.normal(s) * 0.05)(B, S, D)),
            "w1": _w((lambda *s: _rng.normal(s) * 0.05)(D, F) * (D ** -0.5)),
            "b1": _w((lambda *s: _rng.normal(s) * 0.05)(F)),
            "w2": _w((lambda *s: _rng.normal(s) * 0.05)(F, D) * (F ** -0.5)),
            "b2": _w((lambda *s: _rng.normal(s) * 0.05)(D)),
        }
    _B_in = _B_setup()

    return {
        "A_x": _A_in["x"],
        "A_wqkv": _A_in["wqkv"],
        "A_wo": _A_in["wo"],
        "B_x": _B_in["x"],
        "B_w1": _B_in["w1"],
        "B_b1": _B_in["b1"],
        "B_w2": _B_in["w2"],
        "B_b2": _B_in["b2"],
    }

def _fwd_reference(A_x, A_wqkv, A_wo, B_x, B_w1, B_b1, B_w2, B_b2):
    def _A_ref(x, wqkv, wo):
        B, S, D = x.shape
        H = 32; Dh = D // H
        qkv = (lambda x, *d: x.transpose(*d))((x @ wqkv).reshape(B, S, 3, H, Dh), 2, 0, 3, 1, 4)
        q, k, v = qkv[0], qkv[1], qkv[2]
        phi = lambda t: jnp.where(t > 0, t + 1, jnp.exp(t)) + 1e-6
        pq, pk = phi(q), phi(k)
        kv = jnp.einsum("bhsd,bhse->bhde", pk, v)
        z = jnp.einsum("bhsd->bhd", pk)
        num = jnp.einsum("bhqd,bhde->bhqe", pq, kv)
        den = jnp.einsum("bhqd,bhd->bhq", pq, z)[..., None] + 1e-6
        o = num / den
        return (lambda x, *d: x.transpose(*d))(o, 0, 2, 1, 3).reshape(B, S, D) @ wo

    def _B_ref(x, w1, b1, w2, b2):
        y = _layernorm(x, axis=-1)
        h = _gelu(jnp.einsum("bsd,df->bsf", y, w1) + b1)
        return jnp.einsum("bsf,fd->bsd", h, w2) + b2

    x = A_x
    x = x + _A_ref(_layernorm(x, axis=-1), A_wqkv, A_wo)
    x = x + _B_ref(_layernorm(x, axis=-1), B_w1, B_b1, B_w2, B_b2)
    x = x + _A_ref(_layernorm(x, axis=-1), A_wqkv, A_wo)
    x = x + _B_ref(_layernorm(x, axis=-1), B_w1, B_b1, B_w2, B_b2)
    return x


def setup_inputs():
    _inp = _fwd_setup_inputs()
    _gk = jax.random.fold_in(jax.random.key(int.from_bytes(__import__("os").urandom(4), "little")), 2**31 - 1)
    _shapes = [[1, 2048, 576]]
    _dtypes = ['bfloat16']
    _gks = jax.random.split(_gk, len(_shapes))
    _gs = [jax.random.normal(k, s, dtype=jnp.dtype(d)) * 0.05 for k, s, d in zip(_gks, _shapes, _dtypes)]
    _inp["grad_out"] = _gs[0]
    return _inp

def reference(A_x, A_wqkv, A_wo, B_w1, B_b1, B_w2, B_b2, B_x, grad_out):
    _const = dict(B_x=B_x)
    def _f(*_d):
        return _fwd_reference(**{'A_x': _d[0], 'A_wqkv': _d[1], 'A_wo': _d[2], 'B_w1': _d[3], 'B_b1': _d[4], 'B_w2': _d[5], 'B_b2': _d[6], **_const})
    _out, _vjp = jax.vjp(_f, A_x, A_wqkv, A_wo, B_w1, B_b1, B_w2, B_b2)
    _grads = _vjp(grad_out)
    _out0 = jnp.asarray(_out)
    return (_out0, *[jnp.asarray(_g) for _g in _grads])
```

```python
import jax
import jax.numpy as jnp
from jax import lax
import jax.experimental.pallas as pl
import jax.experimental.pallas.tpu as pltpu

S, D, F = 2048, 576, 4608
H, DH = 32, 18
DP = 592
NG, GR, GW = 8, 72, 80
TS = 256
P = TS // 2
NTB = S // TS
HT = S // 2
TF = 256
HF = TF // 2
NC = F // TF
NSUB = 4
SW = HT // NSUB
DK, DM = 256, 288
LN_EPS = 1e-5
PHI_EPS = 1e-6
C0 = 0.7978845608028654
C1 = 0.044715 * C0
bf16, f32 = jnp.bfloat16, jnp.float32


def _nn(a, b):
    return jnp.dot(a, b, preferred_element_type=f32)


def _nt(a, b):
    return lax.dot_general(a, b, (((1,), (1,)), ((), ())), preferred_element_type=f32)


def _win(g):
    return GR * g - 8 * (g % 2)


def _split(a):
    hi = a.astype(bf16)
    lo = (a - hi.astype(f32)).astype(bf16)
    return hi, lo


def _center(x):
    xc = x - jnp.mean(x, axis=0, keepdims=True)
    return xc, jnp.mean(xc * xc, axis=0, keepdims=True)


def _ln_bwd(dy, y, r, k):
    return r * (dy - jnp.mean(dy, axis=0, keepdims=True) - y * (k * jnp.mean(dy * y, axis=0, keepdims=True)))


def _head_rows(a):
    n = a.shape[1]
    b = [jnp.broadcast_to(a[h:h + 1], (8, n)) for h in range(H)]
    sub = lax.broadcasted_iota(jnp.int32, (8, n), 0)
    rows = []
    for j in range(D // 8):
        h0, h1 = (8 * j) // DH, (8 * j + 7) // DH
        rows.append(b[h0] if h0 == h1 else jnp.where(sub < h1 * DH - 8 * j, b[h0], b[h1]))
    return jnp.concatenate(rows, axis=0)


def _gelu(x):
    x2 = x * x
    t = jnp.tanh(x * (C0 + C1 * x2))
    p = 1.0 + t
    h = (0.5 * x) * p
    return h, 0.5 * p + h * (1.0 - t) * (C0 + 3.0 * C1 * x2)


def _quad(a11, a12, a21, a22):
    return jnp.concatenate([jnp.concatenate([a11, a12], axis=1), jnp.concatenate([a21, a22], axis=1)], axis=0)


def _alpha(a11, a12, a21, a22):
    return [a11 + a22, a21 + a22, a11, a22, a11 + a12, a21 - a11, a12 - a22]


def _beta(b11, b12, b21, b22):
    return [b11 + b22, b11, b12 - b22, b21 - b11, b22, b11 + b12, b21 + b22]


def _gamma(c11, c12, c21, c22):
    return [c11 + c22, c21 - c22, c12 + c22, c11 + c21, c12 - c11, c22, c11, c12, c21]


def _beta_t(a):
    return _quad(a[0] + a[1] - a[3] + a[5], a[2] + a[5], a[3] + a[6], a[0] - a[2] + a[4] + a[6])


def _brow(r, T):
    return DK * r + (T if r >= 6 else 0) + (T if r >= 7 else 0)


def _kernel(x_hbm, wqkv_hbm, wo_hbm, w1_hbm, b1_ref, w2_hbm, b2_ref, g_hbm,
            out_hbm, dx_hbm, dwqkv_hbm, dwo_hbm, dw1_hbm, db1_ref, dw2_hbm, db2_ref,
            io, wdu, wqkvT, wo, w1, w2T, xs, ax, ad, gS, uT, qk, yS, pre_s, dw1p, dw2p,
            gh_s, gd_s, aF, bF, aB, bB,
            st, GT, Wp, WpT, kvT, zh, hs, zcol, dWp, dwqk, dwvT, dwo_a, a1, b2c, db2a, sem):
    def cp(src, dst, k):
        return pltpu.make_async_copy(src, dst, sem.at[k])

    def tok(t):
        return pl.ds(pl.multiple_of(t * TS, TS), TS)

    def half(t):
        return pl.ds(pl.multiple_of(t * P, P), P)

    c_x = cp(x_hbm.at[0], io, 0)
    c_wqkv = cp(wqkv_hbm, wdu, 1)
    c_wo = cp(wo_hbm, wo, 2)
    c_w1 = [cp(w1_hbm.at[:, pl.ds(c * TF, TF)], w1.at[c, pl.ds(0, D), :], 3) for c in range(NC)]
    c_w2 = [cp(w2_hbm.at[:, pl.ds(c * TF, TF)], w2T.at[c], 4) for c in range(NC)]
    c_g = cp(g_hbm.at[0], io, 5)
    c_wqkv.start(); c_x.start()

    ones_rows = (lax.broadcasted_iota(jnp.int32, (DP - D, S), 0) < 2).astype(bf16)
    one_row = (lax.broadcasted_iota(jnp.int32, (DP - D, HT), 0) < 1).astype(bf16)
    for l in range(2):
        uT[l, D:DP, :] = ones_rows
        for r in (6, 7):
            yS[l, _brow(r, 80) - 16:_brow(r, 80), :] = one_row
    rj = lax.broadcasted_iota(jnp.int32, (GW, GW), 0)
    ci = lax.broadcasted_iota(jnp.int32, (GW, GW), 1)
    masks = [rj // DH == ci // DH, (rj + (DH - 8)) // DH == (ci + (DH - 8)) // DH]
    hsel = lax.broadcasted_iota(jnp.int32, (H, D), 0) == lax.broadcasted_iota(jnp.int32, (H, D), 1) // DH
    hs[...] = hsel.astype(f32).astype(bf16)
    dwqk[...] = jnp.zeros_like(dwqk)
    dwvT[...] = jnp.zeros_like(dwvT)
    dwo_a[...] = jnp.zeros_like(dwo_a)
    db2a[...] = jnp.zeros_like(db2a)
    b2c[...] = jnp.broadcast_to(b2_ref[...].astype(f32), (128, D)).T
    row0 = lax.broadcasted_iota(jnp.int32, (DP - D, TF), 0) == 0
    for c in range(NC):
        w1[c, D:DP, :] = jnp.where(
            row0, jnp.broadcast_to(b1_ref[:, c * TF:(c + 1) * TF].astype(f32), (DP - D, TF)), 0.0).astype(bf16)

    c_wqkv.wait()
    c_wo.start()
    for c in c_w1 + c_w2:
        c.start()
    wqkvT[...] = wdu[...].T
    wdu[:, 2 * D:3 * D] = wdu[:, D:2 * D]
    c_x.wait()

    def put_beta(dst, T, v, t, extra):
        q = [v[0:DK, 0:P], v[0:DK, P:TS], v[DK:2 * DK, 0:P], v[DK:2 * DK, P:TS]]
        b = _beta(*q) + ([q[1], q[2]] if extra else [])
        for r in range(len(b)):
            dst[_brow(r, T):_brow(r, T) + DK, half(t)] = b[r].astype(bf16)
        dst[_brow(5, T) + DK:_brow(5, T) + DK + D - 2 * DK, half(t)] = v[2 * DK:D, P:TS].astype(bf16)
        dst[_brow(6, T) + DK:_brow(6, T) + DK + D - 2 * DK, half(t)] = v[2 * DK:D, 0:P].astype(bf16)

    def flag_ones(cond):
        return jnp.broadcast_to(jnp.where(cond, 1.0, 0.0).astype(f32), (16, TS)).astype(bf16)

    def phi(z):
        return (jnp.where(z > 0, z + 1.0, jnp.exp(z)) + PHI_EPS).astype(bf16)

    nxt = lambda t: jnp.minimum(t + 1, NTB - 1)
    prv = lambda t: jnp.maximum(t - 1, 0)

    def fwd_a(l):
        GT[l] = jnp.zeros((D, DP), f32)
        onesl = flag_ones(l == 1)

        def s1(t):
            x = jnp.where(l == 0, io[:, tok(t)].astype(f32), _beta_t([ax[r, :, half(t)] for r in range(7)]))
            xs[:, tok(t)] = x
            xc, v = _center(x)
            r = lax.rsqrt(v + LN_EPS)
            st[l, 0:1, tok(t)] = r
            uT[l, 0:D, tok(t)] = (xc * r).astype(bf16)

        def body(t, carry):
            up = uT[l, :, tok(t)]
            pk = phi(_nn(wqkvT[D:2 * D, :], up[0:D]))
            qk[l, D:2 * D, tok(t)] = pk
            dw2p[t] = phi(_nn(wqkvT[0:D, :], up[0:D]))
            GT[l] += _nt(pk, up)
            gb = io[:, tok(t)]
            db2a[...] += _nt(onesl, gb)
            put_beta(gS, 64, gb.astype(f32), t, False)
            ad[:, :, half(t)] = jnp.zeros((7, DM, P), f32)
            s1(nxt(t))
            return carry
        s1(0)
        lax.fori_loop(0, NTB, body, 0)

    def mid_fwd(l):
        G = GT[l]
        gb = G.astype(bf16)
        zcol[l] = jnp.broadcast_to(G[:, D:D + 1], (D, 128))
        sel = (lax.broadcasted_iota(jnp.int32, (H, DP - 512), 1) == D - 512).astype(f32).astype(bf16)
        zh[...] = jnp.where(hsel, _nt(sel, gb[:, 512:DP]), 0.0).astype(bf16)
        rows = []
        for g in range(NG):
            w = _win(g)
            o = GR * g - w
            kv = jnp.where(masks[g % 2], _nt(gb[w:w + GW, 0:D], wqkvT[2 * D + w:2 * D + w + GW, :]), 0.0)
            kvT[l, g] = kv.T[o:o + GR].astype(bf16)
            rows.append(_nn(kv[o:o + GR].astype(bf16), wo[w:w + GW, :]))
        wp = jnp.concatenate(rows, axis=0).astype(bf16)
        Wp[l] = wp
        WpT[...] = wp.T

    def fwd_b(l):
        def s1(t):
            pq = dw2p[t]
            r = _head_rows(1.0 / (_nn(zh[...], pq) + PHI_EPS))
            pqf = pq.astype(f32)
            qk[l, 0:D, tok(t)] = (pqf * r).astype(bf16)
            qk[l, 2 * D:3 * D, tok(t)] = (jnp.minimum(pqf - PHI_EPS, 1.0) * r).astype(bf16)

        def s3(t):
            x = xs[:, tok(t)]
            xc, v = _center(x)
            s = lax.rsqrt(v * (1.0 + LN_EPS) + LN_EPS * LN_EPS)
            st[l, 1:2, tok(t)] = s
            put_beta(yS.at[l], 80, xc * s, t, True)
            xb = x + jnp.tile(b2c[...], (1, TS // 128))
            x11, x12, x21, x22 = xb[0:DM, 0:P], xb[0:DM, P:TS], xb[DM:D, 0:P], xb[DM:D, P:TS]
            zero = jnp.zeros((DM, P), f32)
            for r, val in enumerate([zero, x11 + x21, x12, x21, x22 + x12, zero, zero]):
                ax[r, :, half(t)] = val

        def body(t, carry):
            s3(prv(t))
            xs[:, tok(t)] += _nn(WpT[...], qk[l, 0:D, tok(t)])
            s1(nxt(t))
            return carry
        s1(0)
        lax.fori_loop(0, NTB, body, 0)
        s3(NTB - 1)

    def prep_pre(w, T, c, dst):
        W = lambda r, q: w[c, DK * r:DK * (r + 1), HF * q:HF * (q + 1)].astype(f32)
        al = _alpha(W(0, 0), W(1, 0), W(0, 1), W(1, 1))
        for r in range(7):
            dst[r, :, 0:DK] = al[r].astype(bf16).T
        tl = w[c, 2 * DK:2 * DK + T, :].T
        dst[6, :, DK:DK + T] = tl[0:HF]
        dst[5, :, DK:DK + T] = tl[HF:TF]

    def prep_dy(w, c, dst):
        W = lambda r, q: w[c, DM * r:DM * (r + 1), HF * q:HF * (q + 1)].astype(f32)
        al = _alpha(W(0, 0), W(1, 0), W(0, 1), W(1, 1))
        for r in (0, 1, 4, 5, 6):
            dst[r] = al[r].astype(bf16)

    def prelike(a, bS, T, sl):
        o5, o6 = _brow(5, T), _brow(6, T)
        M = lambda r: _nn(a[r, :, 0:DK], bS[DK * r:DK * (r + 1), sl])
        m2 = M(2); m4 = M(4)
        c12 = _nn(a[6, :, DK:DK + T], bS[o5 + DK:o5 + DK + T, sl]) + m2 + m4
        m1 = M(1); m3 = M(3)
        c21 = _nn(a[5, :, DK:DK + T], bS[o6 + DK:o6 + DK + T, sl]) + m1 + m3
        m0 = M(0)
        c11 = m3 - m4 + m0 + _nn(a[6, :, 0:DK + T], bS[o6:o6 + DK + T, sl])
        c22 = m2 - m1 + m0 + _nn(a[5, :, 0:DK + T], bS[o5:o5 + DK + T, sl])
        return c11, c12, c21, c22

    def dylike(b, w, c, ga, acc, sl):
        for r in range(7):
            al = w[c, 0:DM, 0:HF] if r == 2 else w[c, DM:D, HF:TF] if r == 3 else b[r]
            acc[r, :, sl] += _nn(al, ga[r])

    def dwlike(bS, T, ga, dst, c, first):
        o5, o6 = _brow(5, T), _brow(6, T)
        d = [_nt(bS[DK * r:DK * (r + 1), :], ga[r]) for r in range(5)]
        d5 = _nt(bS[o5:o5 + DK + T, :], ga[5]); d6 = _nt(bS[o6:o6 + DK + T, :], ga[6])
        t0 = d6[DK:] + _nt(bS[o5 + DK:o5 + DK + T, :], ga[7])
        t1 = d5[DK:] + _nt(bS[o6 + DK:o6 + DK + T, :], ga[8])
        d5, d6 = d5[0:DK], d6[0:DK]
        full = jnp.concatenate(
            [jnp.concatenate([d[0] + d[2] + d[4] - d5, d[4] + d6, t0], axis=0),
             jnp.concatenate([d[1] + d5, d[0] + d[1] + d[3] - d6, t1], axis=0)], axis=1)
        tot = (jnp.where(first, 0.0, dst[c].astype(f32)) + full).astype(bf16)
        dst[c] = tot
        return tot

    def out1(c):
        return cp(dw1p.at[c, pl.ds(0, D), :], dw1_hbm.at[:, pl.ds(pl.multiple_of(c * TF, TF), TF)], 3)

    def out2(c):
        return cp(dw2p.at[c], dw2_hbm.at[:, pl.ds(pl.multiple_of(c * TF, TF), TF)], 4)

    def mlp(k):
        def body(c, carry):
            cn = jnp.where(c + 1 < NC, c + 1, 0)
            ps = jnp.where(k == 1, NC, c)

            @pl.when(k < 2)
            def _():
                y = yS.at[k]
                G = {}
                for u in range(NSUB + 1):
                    if u < NSUB:
                        sl = slice(u * SW, (u + 1) * SW)
                        pre = prelike(aF, y, 80, sl)
                        for q in range(4):
                            pre_s[ps, q, :, sl] = pre[q].astype(bf16)
                        G[u] = [v.astype(bf16) for v in _gamma(*[_gelu(p)[0] for p in pre])[0:7]]
                    if u >= 1:
                        dylike(bF, w2T, c, G[u - 1], ax, slice((u - 1) * SW, u * SW))
                prep_pre(w1, 80, cn, aF)
                prep_dy(w2T, cn, bF)

            @pl.when(k > 0)
            def _():
                G = {}
                for u in range(NSUB + 1):
                    if u < NSUB:
                        sl = slice(u * SW, (u + 1) * SW)
                        hg = [_gelu(pre_s[ps, q, :, sl].astype(f32)) for q in range(4)]
                        gh = [v.astype(bf16) for v in _gamma(*[a for a, _ in hg])]
                        dh = prelike(aB, gS, 64, sl)
                        gd = [v.astype(bf16) for v in _gamma(*[d * g for d, (_, g) in zip(dh, hg)])]
                        for r in range(9):
                            gh_s[r, :, sl] = gh[r]
                            gd_s[r, :, sl] = gd[r]
                        G[u] = gd
                    if u == NSUB:
                        dwlike(gS, 64, [gh_s[r] for r in range(9)], dw2p, c, k == 1)
                    if u >= 1:
                        dylike(bB, w1, c, G[u - 1], ad, slice((u - 1) * SW, u * SW))
                d1 = dwlike(yS.at[2 - k], 80, [gd_s[r] for r in range(9)], dw1p, c, k == 1)
                db1_ref[:, pl.ds(pl.multiple_of(c * TF, TF), TF)] = d1[D:D + 1]
                prep_pre(w2T, 64, cn, aB)
                prep_dy(w1, cn, bB)

            @pl.when(k == 2)
            def _():
                out1(c).start()
                out2(c).start()
            return carry
        lax.fori_loop(0, NC, body, 0)

    def c_io(dst, t):
        return cp(io.at[:, tok(t)], dst.at[0, :, tok(t)], 0)

    NB = HT // TS

    def stg(t, r0, n):
        return (pl.ds(pl.multiple_of((t // NB) * 640 + r0, 16), n), pl.ds(pl.multiple_of((t % NB) * TS, TS), TS))

    def bwd_a(l):
        dWp[...] = jnp.zeros_like(dWp)

        def s1(t):
            base = jnp.where(l == 1, io[:, tok(t)].astype(f32), _quad(*[ax[r, :, half(t)] for r in range(4)]))
            dy = _beta_t([ad[r, :, half(t)] for r in range(7)])
            Y = lambda r, n: yS[l, r:r + n, half(t)]
            y = jnp.concatenate(
                [jnp.concatenate([Y(_brow(1, 80), DK), Y(_brow(8, 80), DK), Y(_brow(6, 80) + DK, D - 2 * DK)], axis=0),
                 jnp.concatenate([Y(_brow(7, 80), DK), Y(_brow(4, 80), DK), Y(_brow(5, 80) + DK, D - 2 * DK)], axis=0)],
                axis=1).astype(f32)
            dx = base + _ln_bwd(dy, y, st[l, 1:2, tok(t)], 1.0 + LN_EPS)
            xs[:, tok(t)] = dx
            gS[stg(t, 0, D)] = dx.astype(bf16)

        def body(t, carry):
            dxb = gS[stg(t, 0, D)]
            pqn = qk[l, 0:D, tok(t)]
            dpqn = _nn(Wp[l], dxb)
            c = _nn(hs[...], (dpqn * pqn.astype(f32)).astype(bf16))
            ch, cl = _split(c)
            dWp[...] += _nt(pqn, jnp.concatenate([dxb, ch, cl], axis=0))
            a = qk[l, 2 * D:3 * D, tok(t)].astype(f32)
            qk[l, 0:D, tok(t)] = (a * (dpqn - _head_rows(c) * jnp.tile(zcol[l], (1, TS // 128)))).astype(bf16)
            s1(nxt(t))
            io[:, tok(t)] = _beta_t([ax[r, :, half(t)] for r in range(7)]).astype(bf16)
            ad[:, :, half(t)] = jnp.zeros((7, DM, P), f32)

            @pl.when(l == 1)
            def _():
                c_io(out_hbm, t).start()
            return carry
        s1(0)
        lax.fori_loop(0, NTB, body, 0)

    def mid_bwd(l):
        dw = dWp[:, 0:D].astype(bf16)
        gb = GT[l][:, 0:D].astype(bf16)
        lane = lax.broadcasted_iota(jnp.int32, (D, 128), 1)
        hrow = lax.broadcasted_iota(jnp.int32, (D, 128), 0) // DH
        own = (lane == hrow + 64) | (lane == hrow + 96)
        dz = -jnp.sum(jnp.where(own, dWp[:, 512:640], 0.0), axis=1, keepdims=True)
        zhi, zlo = _split(dz)
        lane = lax.broadcasted_iota(jnp.int32, (D, DP - D), 1)
        a1[:, D:DP] = jnp.where(lane == 0, zhi.astype(f32), jnp.where(lane == 1, zlo.astype(f32), 0.0)).astype(bf16)
        rows = []
        for g in range(NG):
            w = _win(g)
            o = GR * g - w
            dkv = jnp.where(masks[g % 2], _nt(dw[w:w + GW], wo[w:w + GW, :]), 0.0)
            rows.append(_nn(dkv[o:o + GR].astype(bf16), wqkvT[2 * D + w:2 * D + w + GW, :]))
            dwvT[GR * g:GR * (g + 1), :] += _nn(dkv.T[o:o + GR].astype(bf16), gb[w:w + GW])
            dwo_a[GR * g:GR * (g + 1), :] += _nn(kvT[l, g], dw[w:w + GW])
        a = jnp.concatenate(rows, axis=0).astype(bf16)
        a1[:, 0:D] = a
        wdu[:, D:2 * D] = a.T

    def bwd_b(l):
        onesl = flag_ones(l == 1)

        def body(t, carry):
            up = uT[l, :, tok(t)]
            ub = up[0:D]
            dqpk = qk[l, 0:2 * D, tok(t)]
            dpk = _nn(a1[...], up)
            dk = (dpk * jnp.minimum(dqpk[D:2 * D].astype(f32) - PHI_EPS, 1.0)).astype(bf16)
            du = _nn(wdu[:, 0:2 * D], dqpk) + _nn(wdu[:, 2 * D:3 * D], dk)
            dwqk[...] += _nt(ub, jnp.concatenate([dqpk[0:D], dk], axis=0))
            dx = xs[:, tok(t)] + _ln_bwd(du, ub.astype(f32), st[l, 0:1, tok(t)], 1.0)
            for r, val in enumerate([dx[0:DM, 0:P], dx[0:DM, P:TS], dx[DM:D, 0:P], dx[DM:D, P:TS]]):
                ax[r, :, half(t)] = val
            dxb = dx.astype(bf16)
            io[:, tok(t)] = dxb
            db2a[...] += _nt(onesl, dxb)
            put_beta(gS, 64, dx, t, False)

            @pl.when(l == 0)
            def _():
                c_io(dx_hbm, t).start()
            return carry
        lax.fori_loop(0, NTB, body, 0)

    c_dwo = cp(wo, dwo_hbm, 2)
    c_dwv = cp(WpT, dwqkv_hbm.at[:, pl.ds(2 * D, D)], 5)

    def stage(k, carry):
        @pl.when(k < 2)
        def _():
            fwd_a(k)

            @pl.when(k == 0)
            def _():
                c_g.start()
                c_wo.wait()
            mid_fwd(k)
            fwd_b(k)

        @pl.when(k == 0)
        def _():
            for c in c_w1 + c_w2:
                c.wait()
            prep_pre(w1, 80, 0, aF)
            prep_dy(w2T, 0, bF)
            prep_pre(w2T, 64, 0, aB)
            prep_dy(w1, 0, bB)
            c_g.wait()
        mlp(k)

        @pl.when(k > 0)
        def _():
            l = 2 - k
            bwd_a(l)
            mid_bwd(l)

            @pl.when(k == 1)
            def _():
                for t in range(NTB):
                    c_io(out_hbm, t).wait()

            @pl.when(k == 2)
            def _():
                wo[...] = dwo_a[...].astype(bf16)
                c_dwo.start()
                WpT[...] = dwvT[...].astype(bf16).T
                c_dwv.start()
            bwd_b(l)
        return carry
    lax.fori_loop(0, 3, stage, 0)

    c_dwq = []
    for j in range(3):
        cols = pl.ds(384 * j, 384)
        wdu[:, cols] = dwqk[:, cols].astype(bf16)
        c_dwq.append(cp(wdu.at[:, cols], dwqkv_hbm.at[:, cols], 1))
        c_dwq[-1].start()
    db2_ref[...] = db2a[0:1, :].astype(bf16)
    c_dwo.wait()
    c_dwv.wait()
    for c in range(NC):
        out1(c).wait()
        out2(c).wait()
    for t in range(NTB):
        c_io(dx_hbm, t).wait()
    for c in c_dwq:
        c.wait()


@jax.jit
def pallas_interleave_layers__linear_attn_block__mixer_channel_mlp__prompt_kernel(A_x, A_wqkv, A_wo, B_x, B_w1, B_b1, B_w2, B_b2, grad_out):
    anyspec = pl.BlockSpec(memory_space=pl.ANY)
    vspec = pl.BlockSpec(memory_space=pltpu.VMEM)
    V = pltpu.VMEM
    scratch = [
        V((D, S), bf16),
        V((D, 3 * D), bf16),
        V((3 * D, D), bf16),
        V((D, D), bf16),
        V((NC, DP, TF), bf16),
        V((NC, D, TF), bf16),
        V((D, S), f32),
        V((7, DM, HT), f32),
        V((7, DM, HT), f32),
        V((7 * DK + 128, HT), bf16),
        V((2, DP, S), bf16),
        V((2, 3 * D, S), bf16),
        V((2, 9 * DK + 160, HT), bf16),
        V((NC + 1, 4, HF, HT), bf16),
        V((NC, DP, TF), bf16),
        V((NC, D, TF), bf16),
        V((9, HF, HT), bf16),
        V((9, HF, HT), bf16),
        V((7, HF, 384), bf16),
        V((7, DM, HF), bf16),
        V((7, HF, 384), bf16),
        V((7, DM, HF), bf16),
        V((2, 8, S), f32),
        V((2, D, DP), f32),
        V((2, D, D), bf16),
        V((D, D), bf16),
        V((2, NG, GR, GW), bf16),
        V((H, D), bf16),
        V((H, D), bf16),
        V((2, D, 128), f32),
        V((D, 640), f32),
        V((D, 2 * D), f32),
        V((D, D), f32),
        V((D, D), f32),
        V((D, DP), bf16),
        V((D, 128), f32),
        V((16, D), f32),
        pltpu.SemaphoreType.DMA((6,)),
    ]
    sds = jax.ShapeDtypeStruct
    outs = pl.pallas_call(
        _kernel,
        in_specs=[anyspec, anyspec, anyspec, anyspec, vspec, anyspec, vspec, anyspec],
        out_specs=[anyspec, anyspec, anyspec, anyspec, anyspec, vspec, anyspec, vspec],
        out_shape=[sds((1, D, S), bf16), sds((1, D, S), bf16), sds((D, 3 * D), bf16), sds((D, D), bf16),
                   sds((D, F), bf16), sds((1, F), bf16), sds((D, F), bf16), sds((1, D), bf16)],
        scratch_shapes=scratch,
        compiler_params=pltpu.CompilerParams(vmem_limit_bytes=127 * 1024 * 1024),
    )(jnp.swapaxes(A_x, 1, 2), A_wqkv, A_wo, B_w1, B_b1.reshape(1, F), B_w2.T, B_b2.reshape(1, D),
      jnp.swapaxes(grad_out, 1, 2))
    out, dx, dwqkv, dwo, dw1, db1, dw2, db2 = outs
    return (jnp.swapaxes(out, 1, 2), jnp.swapaxes(dx, 1, 2), dwqkv, dwo, dw1, db1.reshape(F), dw2.T,
            db2.reshape(D))
```

```python
import jax
import jax.numpy as jnp
from jax import lax
import jax.experimental.pallas as pl
import jax.experimental.pallas.tpu as pltpu

S, D, F = 2048, 576, 4608
H, DH = 32, 18
DP = 592
NG, GR, GW = 8, 72, 80
TS = 256
P = TS // 2
NTB = S // TS
TF = 256
HF = TF // 2
NC = F // TF
NSUB = 4
BS = NTB // NSUB
SW = BS * P
DK, DM = 256, 288
LN_EPS = 1e-5
PHI_EPS = 1e-6
C0 = 0.7978845608028654
C1 = 0.044715 * C0
bf16, f32, u32 = jnp.bfloat16, jnp.float32, jnp.uint32
CH = 6
R1, RA = D // CH, DM // CH
QCH = [(0, 128), (128, 256), (256, 384), (384, 512), (512, 576)]
ALL = slice(None)
PK = True


def _nn(a, b):
    return jnp.dot(a, b, preferred_element_type=f32)


def _nt(a, b):
    return lax.dot_general(a, b, (((1,), (1,)), ((), ())), preferred_element_type=f32)


def _rows(ref, r0, n, z):
    k = 2 if ref.dtype == u32 else 1
    if z is None:
        return slice(r0 // k, (r0 + n) // k)
    return pl.ds(pl.multiple_of(r0 // k + z * (64 // k), 16 // k), n // k)


def _ld(ref, r0, r1, cols=ALL, z=None):
    v = ref[_rows(ref, r0, r1 - r0, z), cols]
    return pltpu.bitcast(v, bf16) if ref.dtype == u32 else v


def _st(ref, r0, v, cols=ALL, z=None):
    rows = _rows(ref, r0, v.shape[0], z)
    if ref.dtype == u32:
        w = pltpu.bitcast(v.astype(bf16), u32)
        ref[rows, cols] = w
        return lax.bitcast_convert_type(w, f32)
    ref[rows, cols] = v.astype(ref.dtype)
    return v


def _win(g):
    return GR * g - 8 * (g % 2)


def _split(a):
    hi = a.astype(bf16)
    lo = (a - hi.astype(f32)).astype(bf16)
    return hi, lo


def _csum(x):
    return x.reshape(x.shape[0] // 8, 8, x.shape[1]).sum(axis=0)


def _cmean(s):
    return jnp.sum(s, axis=0, keepdims=True) * (1.0 / D)


def _head_rows(row, r0, r1):
    b = {}

    def get(h):
        if h not in b:
            v = row(h)
            b[h] = jnp.broadcast_to(v, (8, v.shape[1]))
        return b[h]
    rows = []
    for j in range(r0 // 8, r1 // 8):
        h0, h1 = (8 * j) // DH, (8 * j + 7) // DH
        if h0 == h1:
            rows.append(get(h0))
        else:
            sub = lax.broadcasted_iota(jnp.int32, get(h0).shape, 0)
            rows.append(jnp.where(sub < h1 * DH - 8 * j, get(h0), get(h1)))
    return jnp.concatenate(rows, axis=0)


def _gate(flag, d, vals, br):
    nr, nc = d.shape[0] // br, d.shape[1] // 128
    blk = [d[br * i:br * (i + 1), 128 * j:128 * (j + 1)] for i in range(nr) for j in range(nc)]
    n = 0
    for v in vals:
        for i in range(v.shape[0] // br):
            for j in range(v.shape[1] // 128):
                blk[n % len(blk)] = jnp.where(flag, v[br * i:br * (i + 1), 128 * j:128 * (j + 1)], blk[n % len(blk)])
                n += 1
    out = jnp.concatenate([jnp.concatenate(blk[nc * i:nc * (i + 1)], axis=1) for i in range(nr)], axis=0)
    if nc * 128 < d.shape[1]:
        out = jnp.concatenate([out, d[0:nr * br, nc * 128:]], axis=1)
    return out


def _gelu(x):
    x2 = x * x
    t = jnp.tanh(x * (C0 + C1 * x2))
    p = 1.0 + t
    h = (0.5 * x) * p
    return h, 0.5 * p + h * (1.0 - t) * (C0 + 3.0 * C1 * x2)


def _quad(a11, a12, a21, a22):
    return jnp.concatenate([jnp.concatenate([a11, a12], axis=1), jnp.concatenate([a21, a22], axis=1)], axis=0)


def _alpha(a11, a12, a21, a22):
    return [a11 + a22, a21 + a22, a11, a22, a11 + a12, a21 - a11, a12 - a22]


def _beta(b11, b12, b21, b22):
    return [b11 + b22, b11, b12 - b22, b21 - b11, b22, b11 + b12, b21 + b22]


def _gamma(c11, c12, c21, c22):
    return [c11 + c22, c21 - c22, c12 + c22, c11 + c21, c12 - c11, c22, c11, c12, c21]


def _beta_t(a):
    return _quad(a[0] + a[1] - a[3] + a[5], a[2] + a[5], a[3] + a[6], a[0] - a[2] + a[4] + a[6])


def _alpha_t(e):
    return _quad(e[0] + e[2] + e[4] - e[5], e[4] + e[6], e[1] + e[5], e[0] + e[1] + e[3] - e[6])


def _prod7(f, t=(0.0, 0.0, 0.0, 0.0)):
    m2 = f(2); m4 = f(4)
    c12 = m2 + m4 if t[1] is None else t[1] + m2 + m4
    m1 = f(1); m3 = f(3)
    c21 = m1 + m3 if t[2] is None else t[2] + m1 + m3
    m0 = f(0)
    c11 = m3 - m4 + m0 + f(6)
    c22 = m2 - m1 + m0 + f(5)
    return (c11 if t[0] is None else c11 + t[0]), c12, c21, (c22 if t[3] is None else c22 + t[3])


def _blocks(a):
    n, m = a.shape[0] // 2, a.shape[1] // 2
    return a[0:n, 0:m], a[0:n, m:], a[n:, 0:m], a[n:, m:]


BT = 49 * 64


def _kernel(x_hbm, wqkv_hbm, wo_hbm, w1_hbm, b1_ref, w2_hbm, b2_ref, g_hbm,
            out_hbm, dx_hbm, dwqkv_hbm, dwo_hbm, dw1_hbm, db1_ref, dw2_hbm, db2_ref,
            io, wl, wdu, wqkvT, wo, w1, w2T, xs, ax, ad, gS, dxs, uT, qk, yS, yr, pre_s, dw1p, dw2p,
            aF, tF, aB, tB,
            st, rr, GT, Wp, WpT, kvT, zh, hs, zcol, dWp, dwqk, dwvT, dwo_a, a1, b2c, db2a, sem):
    def cp(src, dst, k):
        return pltpu.make_async_copy(src, dst, sem.at[k])

    def tok(t):
        return pl.ds(pl.multiple_of(t * TS, TS), TS)

    c_x = [cp(x_hbm.at[0, :, tok(t)], io.at[t], 0) for t in range(NTB)]
    c_wqkv = cp(wqkv_hbm, wl, 1)
    c_wo = cp(wo_hbm, wo, 2)

    def c_w(c):
        cols = pl.ds(pl.multiple_of(c * TF, TF), TF)
        return [cp(w1_hbm.at[:, cols], w1.at[c % 3], 6), cp(w2_hbm.at[:, cols], w2T.at[c % 3], 6)]
    c_g = [cp(g_hbm.at[0, :, tok(t)], io.at[t], 5) for t in range(NTB)]
    c_wqkv.start()
    for c in c_x:
        c.start()

    ones_rows = (lax.broadcasted_iota(jnp.int32, (DP - D, TS), 0) < 2).astype(f32)
    one_row = (lax.broadcasted_iota(jnp.int32, (DP - D, P), 0) < 1).astype(f32)
    for l in range(2):
        for t in range(NTB):
            _st(uT.at[l, t], D, ones_rows)
            for J in range(2):
                _st(yS.at[l, t], BT + 80 * J + 64, one_row)
    st[...] = jnp.zeros_like(st)
    rj = lax.broadcasted_iota(jnp.int32, (GW, GW), 0)
    ci = lax.broadcasted_iota(jnp.int32, (GW, GW), 1)
    masks = [rj // DH == ci // DH, (rj + (DH - 8)) // DH == (ci + (DH - 8)) // DH]
    hsel = lax.broadcasted_iota(jnp.int32, (H, D), 0) == lax.broadcasted_iota(jnp.int32, (H, D), 1) // DH
    _st(hs, 0, hsel.astype(f32))
    dwqk[...] = jnp.zeros_like(dwqk)
    dwvT[...] = jnp.zeros_like(dwvT)
    dwo_a[...] = jnp.zeros_like(dwo_a)
    b2c[...] = jnp.broadcast_to(b2_ref[...].astype(f32), (128, D)).T
    row0 = lax.broadcasted_iota(jnp.int32, (DP - D, TF), 0) == 0

    c_wqkv.wait()
    c_wo.start()
    for c in c_w(0):
        c.start()
    _st(wqkvT, 0, wl[...].T)
    _st(wdu, 0, wl[:, 0:2 * D], slice(0, 2 * D))
    for c in c_x:
        c.wait()

    def ld2(ref, j):
        return jnp.concatenate([_ld(ref, RA * j, RA * (j + 1)), _ld(ref, DM + RA * j, DM + RA * (j + 1))], axis=0)

    def st2(ref, j, v):
        _st(ref, RA * j, v[0:RA])
        _st(ref, DM + RA * j, v[RA:R1])

    def ld1(ref, j, o=0, cols=ALL):
        return _ld(ref, o + R1 * j, o + R1 * (j + 1), cols)

    def comb(acc, j, t):
        return _beta_t([acc[t, r, RA * j:RA * (j + 1), :] for r in range(7)])

    def put_beta(dst, T, get, tq, i, colsum=False):
        if i == 4:
            v = get(tq, 2 * DK, 64, None)
            g = [_st(dst.at[tq], BT + T * J, v[:, P * J:P * (J + 1)]) for J in range(2)]
            if colsum:
                g.append(_st(db2a, 2 * DK, db2a[2 * DK:D] + (v[:, 0:P] + v[:, P:TS])))
            return g
        z = tq % 2
        v = [[[get(tq - z + j, DK * K + 128 * k + 16 * i, 16, z) for j in range(2)] for k in range(2)] for K in range(2)]
        b1 = [[_beta(v[0][k][j][:, 0:P], v[0][k][j][:, P:TS], v[1][k][j][:, 0:P], v[1][k][j][:, P:TS])
               for j in range(2)] for k in range(2)]
        g = []
        for R in range(7):
            b2 = _beta(b1[0][0][R], b1[0][1][R], b1[1][0][R], b1[1][1][R])
            g += [_st(dst.at[tq], 64 * (7 * R + r) + 16 * i, b2[r]) for r in range(7)]
            if colsum and R >= 5:
                for k in range(2):
                    o = DK * (R - 5) + 128 * k + 16 * i
                    g.append(_st(db2a, o, _ld(db2a, o, o + 16, z=z) + b2[5 + k], z=z))
        return g

    def zero_ad(flag, d, j, t):
        z = [jnp.where(flag, d[RA * a:RA * (a + 1), P * b:P * (b + 1)], 0.0) for a in range(2) for b in range(2)]
        for r in range(7):
            ad[t, r, RA * j:RA * (j + 1), :] = z[r % 4]

    def phi(z):
        return (jnp.where(z > 0, z + 1.0, jnp.exp(z)) + PHI_EPS).astype(bf16)

    nxt = lambda t, n=1: jnp.minimum(t + n, NTB - 1)
    prv = lambda t, n=1: jnp.maximum(t - n, 0)

    def fwd_a(l):
        GT[l] = jnp.zeros((D, DP), f32)
        db2a[...] = jnp.zeros_like(db2a)

        def s1a(j, t):
            x = jnp.where(l == 0, ld2(io.at[t], j).astype(f32), comb(ax, j, t))
            st2(xs.at[t], j, x)
            return x

        def s1b(j, t, m):
            xc = ld1(xs.at[t], j) - m
            return xc * xc

        def s1r(t, sv):
            r = lax.rsqrt(_cmean(sv) + LN_EPS)
            st[l, t, 0:1, :] = r
            return r

        def s1c(r0, r1, t, m, r):
            u = (xs[t, r0:r1, :] - m) * r
            return _st(uT.at[l, t], r0, u)

        def body(t, carry):
            flag = t < 0
            tn = nxt(t)
            ub = _ld(uT.at[l, t], 0, D)
            sm = []
            for j in range(CH):
                x = s1a(j, tn)
                sm.append(_csum(x))
                k = _nn(ld1(wqkvT, j, D), ub)
                zero_ad(flag, k, j, t)
                _st(qk.at[l, t], 2 * D + R1 * j, phi(_gate(flag, k, [x], RA)))
            m = _cmean(sum(sm))
            sv = []
            for j in range(CH):
                sq = s1b(j, tn, m)
                sv.append(_csum(sq))
                _st(qk.at[l, t], R1 * j, phi(_gate(flag, _nn(ld1(wqkvT, j), ub), [sq], RA)))
            r = s1r(tn, sum(sv))
            for j, (r0, r1) in enumerate(QCH):
                d = _nt(_ld(qk.at[l, t], 2 * D + r0, 2 * D + r1), _ld(uT.at[l, t], 0, DP))
                u = s1c(r0, r1, tn, m, r)
                b = put_beta(gS, 64, lambda tb, a, n, z: _ld(io.at[tb], a, a + n, z=z).astype(f32), t, j, True)
                GT[l, r0:r1, :] += _gate(flag, d, [u] + b, 8)
            return carry
        m = _cmean(sum([_csum(s1a(j, 0)) for j in range(CH)]))
        r = s1r(0, sum([_csum(s1b(j, 0, m)) for j in range(CH)]))
        s1c(0, D, 0, m, r)
        lax.fori_loop(0, NTB, body, 0)

    def mid_fwd(l):
        G = GT[l]
        gb = G.astype(bf16)
        zcol[l] = jnp.broadcast_to(G[:, D:D + 1], (D, 128))
        sel = (lax.broadcasted_iota(jnp.int32, (H, DP - 512), 1) == D - 512).astype(f32).astype(bf16)
        _st(zh, 0, jnp.where(hsel, _nt(sel, gb[:, 512:DP]), 0.0))
        rows = []
        for g in range(NG):
            w = _win(g)
            o = GR * g - w
            kv = jnp.where(masks[g % 2], _nt(gb[w:w + GW, 0:D], _ld(wqkvT, 2 * D + w, 2 * D + w + GW)), 0.0)
            kvT[l, g] = kv.T[o:o + GR].astype(bf16)
            rows.append(_nn(kv[o:o + GR].astype(bf16), wo[w:w + GW, :]))
        wp = jnp.concatenate(rows, axis=0).astype(bf16)
        _st(Wp.at[l], 0, wp)
        _st(WpT, 0, wp.T)

    def fwd_b(l):
        def den(t):
            rr[l, t] = 1.0 / (_nn(_ld(zh, 0, H), _ld(qk.at[l, t], 0, D)) + PHI_EPS)

        def s1(j, t):
            v = ld1(qk.at[l, t], j).astype(f32) * _head_rows(lambda h: rr[l, t, h:h + 1, :], R1 * j, R1 * (j + 1))
            return _st(qk.at[l, t], D + R1 * j, v)

        def s3a(j, t, m):
            sq = [ld1(xs.at[t], 3 * j + i) - m for i in range(3)]
            return sq[0] * sq[0] + sq[1] * sq[1] + sq[2] * sq[2]

        def s3r(t, m, sv):
            s = lax.rsqrt(_cmean(sv) * (1.0 + LN_EPS) + LN_EPS * LN_EPS)
            st[l, t, 1:2, :] = s
            st[l, t, 2:3, :] = m

        def s3b(i, tq):
            def get(tb, a, n, z):
                y = (_ld(xs.at[tb], a, a + n, z=z) - st[l, tb, 2:3, :]) * st[l, tb, 1:2, :]
                _st(yr.at[l, tb], a, y, z=z)
                return y
            return put_beta(yS.at[l], 80, get, tq, i)

        def body(t, sm):
            flag = t < 0
            tp, tn = prv(t), nxt(t)
            m = _cmean(sm)
            ns, sv = [], []
            for j in range(CH):
                d = _nn(ld2(WpT, j), _ld(qk.at[l, t], D, 2 * D))
                g = [s1(j, tn)]
                if j < 2:
                    g.append(s3a(j, tp, m))
                    sv.append(_csum(g[-1]))
                else:
                    if j == 2:
                        s3r(tp, m, sv[0] + sv[1])
                    for i in {2: [0], 3: [1], 4: [2], 5: [3, 4]}[j]:
                        g += s3b(i, prv(t, 2))
                x = ld2(xs.at[t], j) + _gate(flag, d, g, 8)
                st2(xs.at[t], j, x)
                ns.append(_csum(x))
                xb = x + jnp.tile(ld2(b2c, j), (1, TS // 128))
                x11, x12, x21, x22 = xb[0:RA, 0:P], xb[0:RA, P:TS], xb[RA:R1, 0:P], xb[RA:R1, P:TS]
                zero = jnp.where(flag, x11, 0.0)
                for r, val in enumerate([zero, x11 + x21, x12, x21, x22 + x12, zero, zero]):
                    ax[t, r, RA * j:RA * (j + 1), :] = val
                if j == 0:
                    den(nxt(t, 2))
            return sum(ns)
        den(0)
        den(1)
        for j in range(CH):
            s1(j, 0)
        m = _cmean(lax.fori_loop(0, NTB, body, jnp.zeros((8, TS), f32)))
        s3r(NTB - 1, m, _csum(s3a(0, NTB - 1, m) + s3a(1, NTB - 1, m)))
        for tq in (NTB - 2, NTB - 1):
            for i in range(5):
                s3b(i, tq)

    def prep_pre(w, c, dst, tail, bias):
        a = _alpha(*_blocks(w[c % 3, 0:2 * DK, :].T.astype(f32)))
        g = []
        for R in range(7):
            al = _alpha(*_blocks(a[R]))
            g += [_st(dst.at[7 * R + r], 0, al[r]) for r in range(7)]
        tl = w[c % 3, 2 * DK:D, :]
        if bias:
            b = b1_ref[:, pl.ds(pl.multiple_of(c * TF, TF), TF)].astype(f32)
            tl = jnp.concatenate([tl, jnp.where(row0, jnp.broadcast_to(b, (DP - D, TF)), 0.0).astype(bf16)], axis=0)
        _st(tail, 0, tl.T)
        return g

    def prep_dy(w, c):
        W = lambda r, q: w[c % 3, DM * r:DM * (r + 1), HF * q:HF * (q + 1)].astype(f32)
        return [v.astype(bf16) for v in _alpha(W(0, 0), W(1, 0), W(0, 1), W(1, 1))]

    def bop(bS, p, n):
        return jnp.concatenate([_ld(bS.at[2 * p + z], 64 * n, 64 * (n + 1)) for z in range(2)], axis=0)

    def btail(bS, T, p, J):
        return jnp.concatenate([_ld(bS.at[2 * p + j], BT + T * J, BT + T * (J + 1)) for j in range(2)], axis=1)

    def prelike(a, tail, bS, T, p):
        none = (None,) * 4
        M = lambda R: _quad(*_prod7(lambda r: _nn(_ld(a.at[7 * R + r], 0, 64), bop(bS, p, 7 * R + r)), none))
        t = [_nn(_ld(tail, 0, TF), btail(bS, T, p, J)) for J in range(2)]
        return _prod7(M, (t[0][0:HF], t[1][0:HF], t[0][HF:TF], t[1][HF:TF]))

    def dylike(b, ga, acc, u, gate=None):
        for r in range(7):
            d = _nn(b[r], ga[r])
            if gate is not None:
                d = _gate(gate[0], d, gate[1][7 * r:7 * (r + 1)], 8)
            for i in range(BS):
                acc[BS * u + i, r] += d[:, P * i:P * (i + 1)]

    def gamma2(c):
        g1 = _gamma(*c)[0:7]
        g2 = [v.astype(bf16) for g in g1 for v in _gamma(*_blocks(g))[0:7]]
        return [v.astype(bf16) for v in g1], g2, [v.astype(bf16) for v in c]

    def dw_main(bS, gs, gate=None):
        def e(n):
            d = _nt(jnp.concatenate([g[1][n] for g in gs], axis=1),
                    jnp.concatenate([bop(bS, p, n) for p in range(NSUB)], axis=1))
            return d if gate is None else _gate(gate[0], d, [gate[1][n]], 8)
        return _alpha_t([_alpha_t([e(7 * R + r) for r in range(7)]) for R in range(7)]).T

    def dw_tail(bS, T, gs):
        return _nt(jnp.concatenate([btail(bS, T, p, J) for p in range(NSUB) for J in range(2)], axis=1),
                   jnp.concatenate([_quad(*g[2]) for g in gs], axis=1))

    def dw_put(dst, c, first, r0, v):
        n = v.shape[0]
        tot = (jnp.where(first, 0.0, dst[c, r0:r0 + n, :].astype(f32)) + v).astype(bf16)
        dst[c, r0:r0 + n, :] = tot
        return tot

    def out1(c):
        return cp(dw1p.at[c, pl.ds(0, D), :], dw1_hbm.at[:, pl.ds(pl.multiple_of(c * TF, TF), TF)], 3)

    def out2(c):
        return cp(dw2p.at[c], dw2_hbm.at[:, pl.ds(pl.multiple_of(c * TF, TF), TF)], 4)

    def mlp(k):
        def body(c, carry):
            cn = jnp.where(c + 1 < NC, c + 1, 0)
            ps = jnp.where(k == 1, NC, c)
            flag = c < 0
            for d in c_w(cn):
                d.wait()
            for d in c_w(jnp.where(c + 2 < NC, c + 2, c + 2 - NC)):
                d.start()

            @pl.when(k < 2)
            def _():
                G = {}
                b = prep_dy(w2T, c)
                for u in range(NSUB + 1):
                    if u < NSUB:
                        pre = prelike(aF, tF, yS.at[k], 80, u)
                        for q in range(4):
                            pre_s[ps, q, u] = pre[q].astype(bf16)
                        G[u] = [v.astype(bf16) for v in _gamma(*[_gelu(p)[0] for p in pre])[0:7]]
                    if u >= 1:
                        dylike(b, G[u - 1], ax, u - 1, (flag, prep_pre(w1, cn, aF, tF, True)) if u == NSUB else None)

            @pl.when(k > 0)
            def _():
                gh, gd = [], []
                b = prep_dy(w1, c)
                for u in range(NSUB + 1):
                    if u < NSUB:
                        hg = [_gelu(pre_s[ps, q, u].astype(f32)) for q in range(4)]
                        gh.append(gamma2([a for a, _ in hg]))
                        dh = prelike(aB, tB, gS, 64, u)
                        gd.append(gamma2([d * g for d, (_, g) in zip(dh, hg)]))
                    if u == NSUB:
                        dw_put(dw2p, c, k == 1, 0, dw_main(gS, gh))
                    if u >= 1:
                        dylike(b, gd[u - 1][0], ad, u - 1)
                dw_put(dw1p, c, k == 1, 0, dw_main(yS.at[2 - k], gd, (flag, prep_pre(w2T, cn, aB, tB, False))))
                dw_put(dw2p, c, k == 1, 2 * DK, dw_tail(gS, 64, gh))
                d1 = dw_put(dw1p, c, k == 1, 2 * DK, dw_tail(yS.at[2 - k], 80, gd))
                db1_ref[:, pl.ds(pl.multiple_of(c * TF, TF), TF)] = d1[D - 2 * DK:D - 2 * DK + 1]

            @pl.when(k == 2)
            def _():
                out1(c).start()
                out2(c).start()
            return carry
        lax.fori_loop(0, NC, body, 0)

    def c_io(dst, t):
        return cp(io.at[t], dst.at[0, :, tok(t)], 0)

    def bwd_a(l):
        dWp[...] = jnp.zeros_like(dWp)

        def s1a(j, t):
            dy = comb(ad, j, t)
            st2(xs.at[t], j, dy)
            return dy, dy * ld2(yr.at[l, t], j).astype(f32)

        def s1b(j, t, m1, m2):
            h, o = 2 * (j // 3), R1 * (j % 3)
            base = jnp.where(l == 1, ld1(io.at[t], j).astype(f32),
                             jnp.concatenate([ax[t, h, o:o + R1, :], ax[t, h + 1, o:o + R1, :]], axis=1))
            dx = base + st[l, t, 1:2, :] * (ld1(xs.at[t], j) - m1 - ld1(yr.at[l, t], j).astype(f32) * m2)
            _st(xs.at[t], R1 * j, dx)
            _st(dxs.at[t % 2], R1 * j, dx)
            return dx

        def body(t, carry):
            flag = t < 0
            tn = nxt(t)
            pqn = lambda r0, r1: _ld(qk.at[l, t], D + r0, D + r1)
            dxb = lambda r0, r1: _ld(dxs.at[t % 2], r0, r1)
            s1, s2, dpqn, prod = [], [], [], []
            for j in range(CH):
                d = _nn(ld1(Wp.at[l], j), dxb(0, D))
                if j < 3:
                    (a0, b0), (a1_, b1) = s1a(2 * j, tn), s1a(2 * j + 1, tn)
                    g = [a0 + a1_, b0 + b1]
                    s1.append(_csum(g[0]))
                    s2.append(_csum(g[1]))
                else:
                    if j == 3:
                        m1, m2 = _cmean(sum(s1)), _cmean(sum(s2)) * (1.0 + LN_EPS)
                    g = [s1b(2 * j - 6, tn, m1, m2), s1b(2 * j - 5, tn, m1, m2)]
                dpqn.append(_gate(flag, d, g, RA))
                prod.append((dpqn[j] * pqn(R1 * j, R1 * (j + 1)).astype(f32)).astype(bf16))

            def out(j):
                v = comb(ax, j, t)
                st2(io.at[t], j, v)
                return v

            def dq(j):
                R = _head_rows(lambda h: rr[l, t, h:h + 1, :], R1 * j, R1 * (j + 1))
                a = jnp.minimum(pqn(R1 * j, R1 * (j + 1)).astype(f32) - PHI_EPS * R, R)
                C = _head_rows(lambda h: c[h:h + 1], R1 * j, R1 * (j + 1))
                v = a * (dpqn[j] - C * jnp.tile(ld1(zcol.at[l], j), (1, TS // 128)))
                _st(qk.at[l, t], R1 * j, v)
                return v
            dWp[0:R1, 0:512] += _gate(flag, _nt(pqn(0, R1), dxb(0, 512)), [out(0), out(1), out(2)], RA)
            c = _nn(_ld(hs, 0, H), jnp.concatenate(prod, axis=0))
            dxc = jnp.concatenate([dxb(512, D), *_split(c)], axis=0)
            dWp[R1:2 * R1, 0:512] += _gate(flag, _nt(pqn(R1, 2 * R1), dxb(0, 512)), [out(3), out(4), out(5)], RA)
            for j, js in ((2, [0]), (-1, [1]), (3, [2]), (4, [3, 4]), (5, [5])):
                if j < 0:
                    dWp[0:2 * R1, 512:640] += _gate(flag, _nt(pqn(0, 2 * R1), dxc), [dq(i) for i in js], RA)
                else:
                    dWp[R1 * j:R1 * (j + 1), :] += _gate(
                        flag, _nt(pqn(R1 * j, R1 * (j + 1)), jnp.concatenate([dxb(0, 512), dxc], axis=0)),
                        [dq(i) for i in js], RA)

            @pl.when(l == 1)
            def _():
                c_io(out_hbm, t).start()
            return carry
        p = [s1a(j, 0) for j in range(CH)]
        m1, m2 = _cmean(_csum(sum(a for a, _ in p))), _cmean(_csum(sum(b for _, b in p))) * (1.0 + LN_EPS)
        for j in range(CH):
            s1b(j, 0, m1, m2)
        lax.fori_loop(0, NTB, body, 0)

    def mid_bwd(l):
        dw = dWp[:, 0:D].astype(bf16)
        gb = GT[l][:, 0:D].astype(bf16)
        lane = lax.broadcasted_iota(jnp.int32, (D, 128), 1)
        hrow = lax.broadcasted_iota(jnp.int32, (D, 128), 0) // DH
        own = (lane == hrow + 64) | (lane == hrow + 96)
        dz = -jnp.sum(jnp.where(own, dWp[:, 512:640], 0.0), axis=1, keepdims=True)
        zhi, zlo = _split(dz)
        lane = lax.broadcasted_iota(jnp.int32, (D, DP - D), 1)
        zc = jnp.where(lane == 0, zhi.astype(f32), jnp.where(lane == 1, zlo.astype(f32), 0.0))
        rows = []
        for g in range(NG):
            w = _win(g)
            o = GR * g - w
            dkv = jnp.where(masks[g % 2], _nt(dw[w:w + GW], wo[w:w + GW, :]), 0.0)
            rows.append(_nn(dkv[o:o + GR].astype(bf16), _ld(wqkvT, 2 * D + w, 2 * D + w + GW)))
            dwvT[GR * g:GR * (g + 1), :] += _nn(dkv.T[o:o + GR].astype(bf16), gb[w:w + GW])
            dwo_a[GR * g:GR * (g + 1), :] += _nn(kvT[l, g], dw[w:w + GW])
        a = jnp.concatenate(rows, axis=0)
        _st(a1, 0, jnp.concatenate([a, zc], axis=1))
        _st(wdu, 0, a.astype(bf16).T, slice(2 * D, 3 * D))

    def bwd_b(l):
        def beta_dx(tq, i, skip):
            def get(tb, a, n, z):
                v = _ld(xs.at[tb], a, a + n, z=z)
                return v if skip is None else jnp.where(skip, 0.0, v)
            return put_beta(gS, 64, get, tq, i, True)

        def body(t, carry):
            flag = t < 0
            Q = lambda r0, r1: _ld(qk.at[l, t], r0, r1)
            U = lambda r0, r1: _ld(uT.at[l, t], r0, r1)
            for j in range(CH):
                dpk = _nn(ld1(a1, j), U(0, DP))
                zero_ad(flag, dpk, j, t)
                _st(qk.at[l, t], D + R1 * j, dpk * jnp.minimum(ld1(qk.at[l, t], j, 2 * D).astype(f32) - PHI_EPS, 1.0))
            r = st[l, t, 0:1, :]
            s1, s2 = [], []
            for j in range(CH):
                du = sum(_nn(ld1(wdu, j, 0, slice(a, b)), Q(a, b)) for a, b in ((2 * D, 3 * D), (0, 512), (512, 2 * D)))
                if j < 5:
                    du = _gate(flag, du, beta_dx(prv(t, 2), j, t < 2), 8)
                xs[t, R1 * j:R1 * (j + 1), :] += r * du
                s1.append(_csum(du))
                s2.append(_csum(du * U(R1 * j, R1 * (j + 1)).astype(f32)))
            m1, m2 = r * _cmean(sum(s1)), r * _cmean(sum(s2))
            for j in range(CH):
                dx = ld1(xs.at[t], j) - m1 - U(R1 * j, R1 * (j + 1)).astype(f32) * m2
                _st(xs.at[t], R1 * j, dx)
                _st(io.at[t], R1 * j, dx)
                h, o = 2 * (j // 3), R1 * (j % 3)
                ax[t, h, o:o + R1, :] = dx[:, 0:P]
                ax[t, h + 1, o:o + R1, :] = dx[:, P:TS]
                dwqk[R1 * j:R1 * (j + 1), :] += _gate(flag, _nt(U(R1 * j, R1 * (j + 1)), Q(0, 2 * D)), [dx], 8)

            @pl.when(l == 0)
            def _():
                c_io(dx_hbm, t).start()
            return carry
        lax.fori_loop(0, NTB, body, 0)

        @pl.when(l == 1)
        def _():
            for tq in (NTB - 2, NTB - 1):
                for i in range(5):
                    beta_dx(tq, i, None)

    c_dwo = cp(wo, dwo_hbm, 2)
    c_dwv = cp(wl.at[:, pl.ds(2 * D, D)], dwqkv_hbm.at[:, pl.ds(2 * D, D)], 5)

    def stage(k, carry):
        @pl.when(k < 2)
        def _():
            fwd_a(k)

            @pl.when(k == 0)
            def _():
                for c in c_g:
                    c.start()
                c_wo.wait()
            mid_fwd(k)
            fwd_b(k)

        @pl.when(k == 0)
        def _():
            for c in c_w(0):
                c.wait()
            for c in c_w(1):
                c.start()
            prep_pre(w1, 0, aF, tF, True)
            prep_pre(w2T, 0, aB, tB, False)
            for c in c_g:
                c.wait()
        mlp(k)

        @pl.when(k > 0)
        def _():
            l = 2 - k
            bwd_a(l)
            mid_bwd(l)

            @pl.when(k == 1)
            def _():
                for t in range(NTB):
                    c_io(out_hbm, t).wait()

            @pl.when(k == 2)
            def _():
                wo[...] = dwo_a[...].astype(bf16)
                c_dwo.start()
                wl[:, 2 * D:3 * D] = dwvT[...].astype(bf16).T
                c_dwv.start()
                ones = jnp.ones((16, 128), bf16)
                db2_ref[...] = sum(_nt(ones, v) for v in _split(db2a[...]))[0:1].astype(bf16)
            bwd_b(l)
        return carry
    lax.fori_loop(0, 3, stage, 0)

    c_dwq = []
    for j in range(3):
        cols = pl.ds(384 * j, 384)
        wl[:, cols] = dwqk[:, cols].astype(bf16)
        c_dwq.append(cp(wl.at[:, cols], dwqkv_hbm.at[:, cols], 1))
        c_dwq[-1].start()
    for c in c_w(1):
        c.wait()
    c_dwo.wait()
    c_dwv.wait()
    for c in range(NC):
        out1(c).wait()
        out2(c).wait()
    for t in range(NTB):
        c_io(dx_hbm, t).wait()
    for c in c_dwq:
        c.wait()


@jax.jit
def pallas_interleave_layers__linear_attn_block__mixer_channel_mlp__prompt_kernel(A_x, A_wqkv, A_wo, B_x, B_w1, B_b1, B_w2, B_b2, grad_out):
    anyspec = pl.BlockSpec(memory_space=pl.ANY)
    vspec = pl.BlockSpec(memory_space=pltpu.VMEM)
    V = pltpu.VMEM

    def PB(*s):
        return V(s[:-2] + (s[-2] // 2, s[-1]), u32) if PK else V(s, bf16)
    scratch = [
        V((NTB, D, TS), bf16),
        V((D, 3 * D), bf16),
        PB(D, 3 * D),
        PB(3 * D, D),
        V((D, D), bf16),
        V((3, D, TF), bf16),
        V((3, D, TF), bf16),
        V((NTB, D, TS), f32),
        V((NTB, 7, DM, P), f32),
        V((NTB, 7, DM, P), f32),
        PB(NTB, BT + 128, P),
        PB(2, D, TS),
        PB(2, NTB, DP, TS),
        PB(2, NTB, 3 * D, TS),
        PB(2, NTB, BT + 160, P),
        PB(2, NTB, D, TS),
        V((NC + 1, 4, NSUB, HF, SW), bf16),
        V((NC, DP, TF), bf16),
        V((NC, D, TF), bf16),
        PB(49, 64, 128),
        PB(TF, 80),
        PB(49, 64, 128),
        PB(TF, 64),
        V((2, NTB, 8, TS), f32),
        V((2, NTB, H, TS), f32),
        V((2, D, DP), f32),
        PB(2, D, D),
        PB(D, D),
        V((2, NG, GR, GW), bf16),
        PB(H, D),
        PB(H, D),
        V((2, D, 128), f32),
        V((D, 640), f32),
        V((D, 2 * D), f32),
        V((D, D), f32),
        V((D, D), f32),
        PB(D, DP),
        V((D, 128), f32),
        V((D, 128), f32),
        pltpu.SemaphoreType.DMA((7,)),
    ]
    sds = jax.ShapeDtypeStruct
    outs = pl.pallas_call(
        _kernel,
        in_specs=[anyspec, anyspec, anyspec, anyspec, vspec, anyspec, vspec, anyspec],
        out_specs=[anyspec, anyspec, anyspec, anyspec, anyspec, vspec, anyspec, vspec],
        out_shape=[sds((1, D, S), bf16), sds((1, D, S), bf16), sds((D, 3 * D), bf16), sds((D, D), bf16),
                   sds((D, F), bf16), sds((1, F), bf16), sds((D, F), bf16), sds((1, D), bf16)],
        scratch_shapes=scratch,
        compiler_params=pltpu.CompilerParams(vmem_limit_bytes=128 * 1024 * 1024 - 128 * 1024),
    )(jnp.swapaxes(A_x, 1, 2), A_wqkv, A_wo, B_w1, B_b1.reshape(1, F), B_w2.T, B_b2.reshape(1, D),
      jnp.swapaxes(grad_out, 1, 2))
    out, dx, dwqkv, dwo, dw1, db1, dw2, db2 = outs
    return (jnp.swapaxes(out, 1, 2), jnp.swapaxes(dx, 1, 2), dwqkv, dwo, dw1, db1.reshape(F), dw2.T,
            db2.reshape(D))
```

```python
import jax
import jax.numpy as jnp
from jax import lax
import jax.experimental.pallas as pl
import jax.experimental.pallas.tpu as pltpu

S, D, F = 2048, 576, 4608
H, DH = 32, 18
DP = 592
NG, GR, GW = 8, 72, 80
TS = 256
P = TS // 2
NTB = S // TS
TF = 256
HF = TF // 2
NC = F // TF
NSUB = 4
BS = NTB // NSUB
SW = BS * P
DK, DM = 256, 288
LN_EPS = 1e-5
PHI_EPS = 1e-6
C0 = 0.7978845608028654
C1 = 0.044715 * C0
bf16, f32, u32 = jnp.bfloat16, jnp.float32, jnp.uint32
CH = 6
R1, RA = D // CH, DM // CH
QCH = [(0, 128), (128, 256), (256, 384), (384, 512), (512, 576)]
ALL = slice(None)
PK = True


def _nn(a, b):
    return jnp.dot(a, b, preferred_element_type=f32)


def _nt(a, b):
    return lax.dot_general(a, b, (((1,), (1,)), ((), ())), preferred_element_type=f32)


def _rows(ref, r0, n, z):
    k = 2 if ref.dtype == u32 else 1
    if z is None:
        return slice(r0 // k, (r0 + n) // k)
    return pl.ds(pl.multiple_of(r0 // k + z * (64 // k), 16 // k), n // k)


def _ld(ref, r0, r1, cols=ALL, z=None):
    v = ref[_rows(ref, r0, r1 - r0, z), cols]
    return pltpu.bitcast(v, bf16) if ref.dtype == u32 else v


def _pack(v):
    return pltpu.bitcast(v.astype(bf16), u32)


def _pi(v):
    h = [jnp.concatenate([v[r + o:r + o + 8] for r in range(0, v.shape[0], 16)], axis=0) for o in (0, 8)]
    return pltpu.pack_elementwise(h, packed_dtype=bf16)


def _ui(w):
    w = w if w.dtype == u32 else pltpu.bitcast(w, u32)
    h = [pltpu.unpack_elementwise(w, index=i, packed_dtype=bf16, unpacked_dtype=f32) for i in range(2)]
    return jnp.concatenate([x[r:r + 8] for r in range(0, w.shape[0], 8) for x in h], axis=0)


def _b16(v):
    return pltpu.bitcast(_pi(v), bf16)


def _st(ref, r0, v, cols=ALL, z=None):
    if ref.dtype == u32:
        w = v if v.dtype == u32 else _pack(v)
        ref[_rows(ref, r0, 2 * w.shape[0], z), cols] = w
        return lax.bitcast_convert_type(w, f32)
    ref[_rows(ref, r0, v.shape[0], z), cols] = v.astype(ref.dtype)
    return v


def _win(g):
    return GR * g - 8 * (g % 2)


def _split(a):
    hi = a.astype(bf16)
    lo = (a - hi.astype(f32)).astype(bf16)
    return hi, lo


def _csum(x):
    return x.reshape(x.shape[0] // 8, 8, x.shape[1]).sum(axis=0)


def _cmean(s):
    return jnp.sum(s, axis=0, keepdims=True) * (1.0 / D)


def _head_rows(row, r0, r1):
    b = {}

    def get(h):
        if h not in b:
            v = row(h)
            b[h] = jnp.broadcast_to(v, (8, v.shape[1]))
        return b[h]
    rows = []
    for j in range(r0 // 8, r1 // 8):
        h0, h1 = (8 * j) // DH, (8 * j + 7) // DH
        if h0 == h1:
            rows.append(get(h0))
        else:
            sub = lax.broadcasted_iota(jnp.int32, get(h0).shape, 0)
            rows.append(jnp.where(sub < h1 * DH - 8 * j, get(h0), get(h1)))
    return jnp.concatenate(rows, axis=0)


def _gate(flag, d, vals, br, spread=False):
    nr, nc = d.shape[0] // br, d.shape[1] // 128
    blk = [d[br * i:br * (i + 1), 128 * j:128 * (j + 1)] for i in range(nr) for j in range(nc)]
    vs = [v[br * i:br * (i + 1), 128 * j:128 * (j + 1)]
          for v in vals for i in range(v.shape[0] // br) for j in range(v.shape[1] // 128)]
    for n, v in enumerate(vs):
        m = n * len(blk) // len(vs) if spread else n % len(blk)
        blk[m] = jnp.where(flag, v, blk[m])
    out = jnp.concatenate([jnp.concatenate(blk[nc * i:nc * (i + 1)], axis=1) for i in range(nr)], axis=0)
    if nc * 128 < d.shape[1]:
        out = jnp.concatenate([out, d[0:nr * br, nc * 128:]], axis=1)
    return out


def _gelu(x):
    x2 = x * x
    s = 0.5 * jnp.tanh(x * (C0 + C1 * x2)) + 0.5
    h = x * s
    return h, s + h * (1.0 - s) * (2.0 * C0 + 6.0 * C1 * x2)


def _quad(a11, a12, a21, a22):
    return jnp.concatenate([jnp.concatenate([a11, a12], axis=1), jnp.concatenate([a21, a22], axis=1)], axis=0)


def _alpha(a11, a12, a21, a22):
    return [a11 + a22, a21 + a22, a11, a22, a11 + a12, a21 - a11, a12 - a22]


def _beta(b11, b12, b21, b22):
    return [b11 + b22, b11, b12 - b22, b21 - b11, b22, b11 + b12, b21 + b22]


def _gamma(c11, c12, c21, c22):
    return [c11 + c22, c21 - c22, c12 + c22, c11 + c21, c12 - c11, c22, c11, c12, c21]


def _beta_t(a):
    return _quad(a[0] + a[1] - a[3] + a[5], a[2] + a[5], a[3] + a[6], a[0] - a[2] + a[4] + a[6])


def _alpha_t(e):
    return _quad(e[0] + e[2] + e[4] - e[5], e[4] + e[6], e[1] + e[5], e[0] + e[1] + e[3] - e[6])


def _prod7(f, t=None):
    m2 = f(2); m4 = f(4)
    c12 = m2 + m4 if t is None else m2 + m4 + t(1)
    m1 = f(1); m3 = f(3)
    c21 = m1 + m3 if t is None else m1 + m3 + t(2)
    m0 = f(0)
    c11 = m3 - m4 + m0 + f(6)
    c11 = c11 if t is None else c11 + t(0)
    c22 = m2 - m1 + m0 + f(5)
    c22 = c22 if t is None else c22 + t(3)
    return c11, c12, c21, c22


ORD = (2, 4, 1, 3, 0, 6, 5)
DB = 0
LAG = 12
DWG = (0, 2, 4, 5)
DWL = 4


def _w32(v):
    return lax.bitcast_convert_type(pltpu.bitcast(v, u32), f32)


def _blocks(a):
    n, m = a.shape[0] // 2, a.shape[1] // 2
    return a[0:n, 0:m], a[0:n, m:], a[n:, 0:m], a[n:, m:]


BT = 49 * 64


def _kernel(x_hbm, wqkv_hbm, wo_hbm, w1_hbm, b1_ref, w2_hbm, b2_ref, g_hbm,
            out_hbm, dx_hbm, dwqkv_hbm, dwo_hbm, dw1_hbm, db1_ref, dw2_hbm, db2_ref,
            io, wt, wdu, wqkvT, wo, w1, w2T, xs, ax, ad, gS, dxs, uT, qk, yS, yr, pre_s, dw1p, dw2p,
            aF, tF, aB, tB,
            st, rr, GT, Wp, WpT, kvT, zh, hs, zcol, dWp, dwqk, dwvT, dwo_a, a1, b2c, db2a, sem):
    def cp(src, dst, k):
        return pltpu.make_async_copy(src, dst, sem.at[k])

    def tok(t):
        return pl.ds(pl.multiple_of(t * TS, TS), TS)

    c_x = [cp(x_hbm.at[0, :, tok(t)], io.at[t], 0 if t > 1 else 5) for t in range(NTB)]

    def stg(j, c0, n):
        return (wt if n == 64 else dw1p.at[j, pl.ds(0, D), pl.ds(0, n)]), pl.ds(c0, n)
    wq = [stg(j, TF * j, TF) for j in range(6)] + [stg(6, 6 * TF, 128), stg(7, 6 * TF + 128, 64)]
    c_wqkv = [cp(wqkv_hbm.at[:, cols], buf, (1, 1, 1, 3, 3, 4, 4, 4)[j]) for j, (buf, cols) in enumerate(wq)]
    c_wo = cp(wo_hbm, wo, 2)

    def c_w(c, sl=None):
        cols = pl.ds(pl.multiple_of(c * TF, TF), TF)
        sl = c if sl is None else sl
        return [cp(w1_hbm.at[:, cols], w1.at[sl], 6), cp(w2_hbm.at[:, cols], w2T.at[sl], 6)]
    c_g = [cp(g_hbm.at[0, :, tok(t)], io.at[t], 5) for t in range(NTB)]
    for c in c_wqkv[0:5] + c_x[0:2] + c_wqkv[5:8] + c_x[2:]:
        c.start()

    ones_rows = (lax.broadcasted_iota(jnp.int32, (DP - D, TS), 0) < 2).astype(f32)
    one_row = (lax.broadcasted_iota(jnp.int32, (DP - D, P), 0) < 1).astype(f32)
    for l in range(2):
        for t in range(NTB):
            _st(uT.at[l, t], D, ones_rows)
            for J in range(2):
                _st(yS.at[l, t], BT + 80 * J + 64, one_row)
    st[...] = jnp.zeros_like(st)
    rj = lax.broadcasted_iota(jnp.int32, (GW, GW), 0)
    ci = lax.broadcasted_iota(jnp.int32, (GW, GW), 1)
    masks = [rj // DH == ci // DH, (rj + (DH - 8)) // DH == (ci + (DH - 8)) // DH]
    hsel = lax.broadcasted_iota(jnp.int32, (H, D), 0) == lax.broadcasted_iota(jnp.int32, (H, D), 1) // DH
    _st(hs, 0, hsel.astype(f32))
    GT[...] = jnp.zeros_like(GT)
    b2c[...] = jnp.broadcast_to(b2_ref[...].astype(f32), (128, D)).T
    row0 = lax.broadcasted_iota(jnp.int32, (DP - D, TF), 0) == 0

    for js in ((0, 1, 2), (3, 4), (5, 6, 7)):
        for j in js:
            c_wqkv[j].wait()
        for j in js:
            buf, cols = wq[j]
            _st(wqkvT, cols.start, buf[...].T)
            n = min(TF, 2 * D - TF * j)
            if n > 0:
                _st(wdu, 0, buf[:, 0:n], slice(TF * j, TF * j + n))
        if js[0] == 0:
            dwqk[...] = jnp.zeros_like(dwqk)
        if js[0] == 3:
            dwvT[...] = jnp.zeros_like(dwvT)
        if js[0] == 5:
            dwo_a[...] = jnp.zeros_like(dwo_a)
    for c in c_x[0:2]:
        c.wait()

    def ld2(ref, j):
        return jnp.concatenate([_ld(ref, RA * j, RA * (j + 1)), _ld(ref, DM + RA * j, DM + RA * (j + 1))], axis=0)

    def st2(ref, j, v):
        _st(ref, RA * j, v[0:RA])
        _st(ref, DM + RA * j, v[RA:R1])

    def ld1(ref, j, o=0, cols=ALL):
        return _ld(ref, o + R1 * j, o + R1 * (j + 1), cols)

    def comb(acc, j, t):
        return _beta_t([acc[t, r, RA * j:RA * (j + 1), :] for r in range(7)])

    def put_beta(dst, T, get, tq, i, colsum=False):
        if i == 4:
            w = get(tq, 2 * DK, 64, None)
            g = [_st(dst.at[tq], BT + T * J, w[:, P * J:P * (J + 1)]) for J in range(2)]
            if colsum:
                v = _ui(w)
                g.append(_st(db2a, 2 * DK, db2a[2 * DK:D] + (v[:, 0:P] + v[:, P:TS])))
            return g
        z = tq % 2
        v = [[[_ui(get(tq - z + j, DK * K + 128 * k + 16 * i, 16, z)) for j in range(2)] for k in range(2)] for K in range(2)]
        b1 = [[_beta(v[0][k][j][:, 0:P], v[0][k][j][:, P:TS], v[1][k][j][:, 0:P], v[1][k][j][:, P:TS])
               for j in range(2)] for k in range(2)]
        g = []
        for R in range(7):
            b2 = _beta(b1[0][0][R], b1[0][1][R], b1[1][0][R], b1[1][1][R])
            g += [_st(dst.at[tq], 64 * (7 * R + r) + 16 * i, _pi(b2[r])) for r in range(7)]
            if colsum and R >= 5:
                for k in range(2):
                    o = DK * (R - 5) + 128 * k + 16 * i
                    g.append(_st(db2a, o, _ld(db2a, o, o + 16, z=z) + b2[5 + k], z=z))
        return g

    def beta_io(tq, i, skip=None):
        def get(tb, a, n, z):
            w = pltpu.bitcast(_ld(io.at[tb], a, a + n, z=z), u32)
            return w if skip is None else jnp.where(skip, jnp.uint32(0), w)
        return put_beta(gS, 64, get, tq, i, True)

    def zero_ad(flag, d, j, t):
        z = [jnp.where(flag, d[RA * a:RA * (a + 1), P * b:P * (b + 1)], 0.0) for a in range(2) for b in range(2)]
        for r in range(7):
            ad[t, r, RA * j:RA * (j + 1), :] = z[r % 4]

    def phi(z):
        return (jnp.where(z > 0, z + 1.0, jnp.exp(z)) + PHI_EPS).astype(bf16)

    nxt = lambda t, n=1: jnp.minimum(t + n, NTB - 1)
    prv = lambda t, n=1: jnp.maximum(t - n, 0)

    def fwd_a(l):
        db2a[...] = jnp.zeros_like(db2a)

        def s1a(j, t):
            x = jnp.where(l == 0, ld2(io.at[t], j).astype(f32), comb(ax, j, t))
            st2(xs.at[t], j, x)
            return x

        def s1b(j, t, m):
            xc = ld1(xs.at[t], j) - m
            return xc * xc

        def s1r(t, sv):
            r = lax.rsqrt(_cmean(sv) + LN_EPS)
            st[l, t, 0:1, :] = r
            return r

        def s1c(r0, r1, t, m, r):
            u = (xs[t, r0:r1, :] - m) * r
            return _st(uT.at[l, t], r0, u)

        def body(t, carry):
            flag = t < 0
            tn = nxt(t)

            @pl.when((l == 0) & (t == 1))
            def _():
                for c in c_x[2:]:
                    c.wait()
                for c in [c_wo] + c_w(0):
                    c.start()
            ub = _ld(uT.at[l, t], 0, D)
            sm = []
            for j in range(CH):
                x = s1a(j, tn)
                sm.append(_csum(x))
                k = _nn(ld1(wqkvT, j, D), ub)
                zero_ad(flag, k, j, t)
                _st(qk.at[l, t], 2 * D + R1 * j, phi(_gate(flag, k, [x], RA)))
            m = _cmean(sum(sm))
            sv = []
            for j in range(CH):
                sq = s1b(j, tn, m)
                sv.append(_csum(sq))
                _st(qk.at[l, t], R1 * j, phi(_gate(flag, _nn(ld1(wqkvT, j), ub), [sq], RA)))
            r = s1r(tn, sum(sv))
            for j, (r0, r1) in enumerate(QCH):
                d = _nt(_ld(qk.at[l, t], 2 * D + r0, 2 * D + r1), _ld(uT.at[l, t], 0, DP))
                u = s1c(r0, r1, tn, m, r)
                b = beta_io(t, j)
                GT[l, r0:r1, :] += _gate(flag, d, [u] + b, 8)
            return carry
        m = _cmean(sum([_csum(s1a(j, 0)) for j in range(CH)]))
        r = s1r(0, sum([_csum(s1b(j, 0, m)) for j in range(CH)]))
        s1c(0, D, 0, m, r)
        lax.fori_loop(0, NTB, body, 0)

    def mid_fwd(l):
        G = GT[l]
        gb = G.astype(bf16)
        zcol[l] = jnp.broadcast_to(G[:, D:D + 1], (D, 128))
        sel = (lax.broadcasted_iota(jnp.int32, (H, DP - 512), 1) == D - 512).astype(f32).astype(bf16)
        _st(zh, 0, jnp.where(hsel, _nt(sel, gb[:, 512:DP]), 0.0))
        win = [(_win(g), GR * g - _win(g)) for g in range(NG)]
        kv = [jnp.where(masks[g % 2], _nt(gb[w:w + GW, 0:D], _ld(wqkvT, 2 * D + w, 2 * D + w + GW)), 0.0)
              for g, (w, o) in enumerate(win)]
        rows = [_nn(kv[g][o:o + GR].astype(bf16), wo[w:w + GW, :]) for g, (w, o) in enumerate(win)]
        for g, (w, o) in enumerate(win):
            kvT[l, g] = kv[g].T[o:o + GR].astype(bf16)
        wp = jnp.concatenate(rows, axis=0).astype(bf16)
        _st(Wp.at[l], 0, wp)
        _st(WpT, 0, wp.T)

    def fwd_b(l):
        def den(t):
            rr[l, t] = 1.0 / (_nn(_ld(zh, 0, H), _ld(qk.at[l, t], 0, D)) + PHI_EPS)

        def s1(j, t):
            v = ld1(qk.at[l, t], j).astype(f32) * _head_rows(lambda h: rr[l, t, h:h + 1, :], R1 * j, R1 * (j + 1))
            return _st(qk.at[l, t], D + R1 * j, v)

        def s3a(j, t, m):
            sq = [ld1(xs.at[t], 3 * j + i) - m for i in range(3)]
            return sq[0] * sq[0] + sq[1] * sq[1] + sq[2] * sq[2]

        def s3r(t, m, sv):
            s = lax.rsqrt(_cmean(sv) * (1.0 + LN_EPS) + LN_EPS * LN_EPS)
            st[l, t, 1:2, :] = s
            st[l, t, 2:3, :] = m

        def s3b(i, tq):
            def get(tb, a, n, z):
                y = (_ld(xs.at[tb], a, a + n, z=z) - st[l, tb, 2:3, :]) * st[l, tb, 1:2, :]
                _st(yr.at[l, tb], a, y, z=z)
                return yr.at[l, tb][_rows(yr, a, n, z), :]
            return put_beta(yS.at[l], 80, get, tq, i)

        def body(t, sm):
            flag = t < 0
            tp, tn = prv(t), nxt(t)
            m = _cmean(sm)
            ns, sv = [], []
            for j in range(CH):
                d = _nn(ld2(WpT, j), _ld(qk.at[l, t], D, 2 * D))
                g = [s1(j, tn)]
                if j < 2:
                    g.append(s3a(j, tp, m))
                    sv.append(_csum(g[-1]))
                else:
                    if j == 2:
                        s3r(tp, m, sv[0] + sv[1])
                    for i in {2: [0], 3: [1], 4: [2], 5: [3, 4]}[j]:
                        g += s3b(i, prv(t, 2))
                x = ld2(xs.at[t], j) + _gate(flag, d, g, 8)
                st2(xs.at[t], j, x)
                ns.append(_csum(x))
                xb = x + jnp.tile(ld2(b2c, j), (1, TS // 128))
                x11, x12, x21, x22 = xb[0:RA, 0:P], xb[0:RA, P:TS], xb[RA:R1, 0:P], xb[RA:R1, P:TS]
                zero = jnp.where(flag, x11, 0.0)
                for r, val in enumerate([zero, x11 + x21, x12, x21, x22 + x12, zero, zero]):
                    ax[t, r, RA * j:RA * (j + 1), :] = val
                if j == 0:
                    den(nxt(t, 2))
            return sum(ns)
        den(0)
        den(1)
        for j in range(CH):
            s1(j, 0)
        m = _cmean(lax.fori_loop(0, NTB, body, jnp.zeros((8, TS), f32)))
        s3r(NTB - 1, m, _csum(s3a(0, NTB - 1, m) + s3a(1, NTB - 1, m)))
        for tq in (NTB - 2, NTB - 1):
            for i in range(5):
                s3b(i, tq)

    def prep_pre(w, c, sl, dst, tail, bias):
        a = _alpha(*_blocks(_ui(_ui(w[sl, 0:2 * DK, :].T).astype(bf16))))
        g = []
        for R in range(7):
            al = _alpha(*_blocks(a[R]))
            g += [_st(dst.at[7 * R + r], 0, _pi(al[r])) for r in range(7)]
        tl = w[sl, 2 * DK:D, :]
        if bias:
            b = b1_ref[:, pl.ds(pl.multiple_of(c * TF, TF), TF)].astype(f32)
            tl = jnp.concatenate([tl, jnp.where(row0, jnp.broadcast_to(b, (DP - D, TF)), 0.0).astype(bf16)], axis=0)
        _st(tail, 0, _ui(tl.T))
        return g

    def prep_dy(w, sl):
        W = lambda r, q: _ui(w[sl, DM * r:DM * (r + 1), HF * q:HF * (q + 1)])
        return [_b16(v) for v in _alpha(W(0, 0), W(1, 0), W(0, 1), W(1, 1))]

    def bop(bS, p, n):
        return jnp.concatenate([_ld(bS.at[2 * p + z], 64 * n, 64 * (n + 1)) for z in range(2)], axis=0)

    def btail(bS, T, p, J):
        return jnp.concatenate([_ld(bS.at[2 * p + j], BT + T * J, BT + T * (J + 1)) for j in range(2)], axis=1)

    hist = []

    def prelike(a, tail, bS, T, p, flag=None, work=None, pre=None):
        def M(R):
            i = ORD.index(R)
            if pre is not None:
                pre(i)

            def f(r):
                d = _nn(_ld(a.at[7 * R + r], 0, 64), bop(bS, p, 7 * R + r))
                g = work(7 * i + ORD.index(r)) if work is not None else []
                hist.append(d[0:8])
                return _gate(flag, d, g, 8) if g else d
            return _quad(*_prod7(f))
        return _prod7(M, lambda q: _nn(_ld(tail, HF * (q // 2), HF * (q // 2 + 1)), btail(bS, T, p, q % 2)))

    def dy1(b, ga, acc, u, r, flag=None, g=()):
        d = _nn(b[r], ga[r])
        hist.extend([d[96 * i:96 * i + 8, 0:128] for i in range(3)])
        if len(g):
            d = _gate(flag, d, g, 8, True)
        for i in range(BS):
            acc[BS * u + i, r] += d[:, P * i:P * (i + 1)]
        return d

    def dylike(b, ga, acc, u, gate=None):
        for r in range(7):
            dy1(b, ga, acc, u, r, *(() if gate is None else (gate[0], gate[1][7 * r:7 * (r + 1)])))

    def dw_main(bS, g1, put, flag, gate=None):
        E, pend = {}, []
        for m, R in enumerate((4, 6, 1, 5, 0, 2, 3)):
            ops = [_gamma(*_blocks(g[R]))[0:7] for g in g1]
            e = []
            for r in range(7):
                n = 7 * R + r
                d = _nt(_b16(jnp.concatenate([o[r] for o in ops], axis=1)),
                        jnp.concatenate([bop(bS, p, n) for p in range(NSUB)], axis=1))
                g = [] if gate is None else [gate[7 * m + r]]
                if r >= 3 and pend:
                    g.append(pend[0][64 * (r - 3):64 * (r - 2)])
                e.append(_gate(flag, d, g, 8) if g else d)
            E[R] = _alpha_t(e)
            pend = []
            if R == 6:
                pend = [put(1, 0, (E[4] + E[6]).T)]
            if R == 5:
                pend = [put(0, 1, (E[1] + E[5]).T)]
            if R == 2:
                pend = [put(0, 0, (E[0] + E[2] + E[4] - E[5]).T)]
            if R == 3:
                put(1, 1, (E[0] + E[1] + E[3] - E[6]).T)

    def dw_tail(bS, T, gs):
        return _nt(jnp.concatenate([btail(bS, T, p, J) for p in range(NSUB) for J in range(2)], axis=1),
                   jnp.concatenate([_quad(*g) for g in gs], axis=1))

    def dw_put(dst, c, first, r0, v, c0=0):
        idx = (c, slice(r0, r0 + v.shape[0]), slice(c0, c0 + v.shape[1]))
        tot = jnp.where(first, 0.0, dst[idx].astype(f32)) + v
        dst[idx] = tot.astype(bf16)
        return tot

    def out1(c):
        return cp(dw1p.at[c, pl.ds(0, D), :], dw1_hbm.at[:, pl.ds(pl.multiple_of(c * TF, TF), TF)], 3)

    def out2(c):
        return cp(dw2p.at[c], dw2_hbm.at[:, pl.ds(pl.multiple_of(c * TF, TF), TF)], 4)

    def mlp(k):
        def body(c, sl):
            cn = jnp.where(c + 1 < NC, c + 1, 0)
            ps = jnp.where(k == 1, NC, c)
            flag = c < 0

            def pres(q, u, n, t=None):
                w = pre_s[ps, q, u, 8 * (n // 2):8 * (n // 2 + 1), P * (n % 2):P * (n % 2 + 1)]
                if t is not None:
                    w = jnp.where(flag, t, w)
                return _ui(w)
            for d in c_w(cn, sl[1]):
                d.wait()
            for d in c_w(jnp.where(c + 2 < NC, c + 2, c + 2 - NC), sl[2]):
                d.start()

            @pl.when(k < 2)
            def _():
                pre, G = {}, {}
                b = prep_dy(w2T, sl[0])

                def piece(u, n):
                    i, j = n // 2, n % 2
                    G[u, n] = [_pi(v) for v in _gamma(*[_gelu(pres(q, u, n))[0] for q in range(4)])[0:7]]
                    return [lax.bitcast_convert_type(v, f32) for v in G[u, n]]

                def gall(u):
                    return [pltpu.bitcast(jnp.concatenate(
                        [jnp.concatenate([G[u, 2 * i + j][r] for j in range(2)], axis=1) for i in range(8)], axis=0), bf16)
                        for r in range(7)]
                for s in range(NSUB + 2):
                    ga = gall(s - 2) if s >= 2 else None
                    if s < NSUB:
                        pre[s] = prelike(aF, tF, yS.at[k], 80, s, flag,
                                         (lambda n: piece(s - 1, n // 3) if n % 3 == 2 else []) if s >= 1 else None,
                                         (lambda i: dy1(b, ga, ax, s - 2, i)) if s >= 2 else None)
                        for q in range(4):
                            _st(pre_s.at[ps, q, s], 0, _pi(pre[s][q]))
                    elif s == NSUB:
                        for r in range(7):
                            dy1(b, ga, ax, s - 2, r, flag,
                                [v for n in range(16 * r // 7, 16 * (r + 1) // 7) for v in piece(s - 1, n)])
                    else:
                        dylike(b, ga, ax, s - 2, (flag, prep_pre(w1, cn, sl[1], aF, tF, True)))

            @pl.when(k > 0)
            def _():
                dh, G, HG = {}, {}, {}
                b = prep_dy(w1, sl[0])

                def pa(u, n, t=None):
                    HG[u, n] = [_gelu(pres(q, u, n, t)) for q in range(4)]
                    return [g for _, g in HG[u, n]]

                def pb(u, n):
                    i, j = n // 2, n % 2
                    if (u, n) not in HG:
                        pa(u, n)
                    dp = [d[16 * i:16 * (i + 1), P * j:P * (j + 1)] * g for d, (_, g) in zip(dh[u], HG[u, n])]
                    G[u, n] = ([_pi(v) for v in _gamma(*dp)] + [a for a, _ in HG[u, n]] + dp + [_pi(a) for a, _ in HG[u, n]])
                    return [lax.bitcast_convert_type(v, f32) for v in G[u, n][0:9 if DB & 1 else 7] + (G[u, n][17:21] if DB & 2 else [])]

                def gall(u, rs):
                    o = [jnp.concatenate([jnp.concatenate([G[u, 2 * i + j][r] for j in range(2)], axis=1)
                                          for i in range(8)], axis=0) for r in rs]
                    return [pltpu.bitcast(v, bf16) if v.dtype == u32 else v for v in o]
                jobs = [[(pa, 0, n) for n in range(0, 16, 2)]] + [[(pb, u, n) for n in range(16)] for u in range(NSUB)]
                dys = [[], [], [(0, r) for r in range(4)], [(0, 4), (0, 5), (0, 6), (1, 0)],
                       [(1, r) for r in range(1, 7)] + [(2, r) for r in range(7)]]

                def work(s, n, tot):
                    J = jobs[s]
                    return [v for f, u, i in J[len(J) * n // tot:len(J) * (n + 1) // tot] for v in f(u, i)]

                def dy(u, r, g=()):
                    dy1(b, {r: gall(u, [r])[0]}, ad, u, r, flag, g)
                for s in range(NSUB + 1):
                    if s < NSUB:
                        dh[s] = prelike(aB, tB, gS, 64, s, flag, lambda n: work(s, n, 49),
                                        lambda i: [dy(*x) for x in dys[s][i // 2:i // 2 + 1]] if i % 2 == 0 else None)
                    else:
                        for m, x in enumerate(dys[s]):
                            dy(*x, work(s, m, len(dys[s])))
                gh = [gall(u, range(17, 21)) for u in range(NSUB)]
                gd = [gall(u, (6, 7, 8, 5)) for u in range(NSUB)]
                dylike(b, gall(NSUB - 1, range(7)), ad, NSUB - 1)
                put = lambda dst: lambda i, j, v: dw_put(dst, c, k == 1, DK * i, v, HF * j)
                uq = lambda v, R: _ui(jnp.where(flag, jnp.uint32(R), pltpu.bitcast(v, u32)))
                dw_main(gS, [[_gamma(*[uq(v, R) for v in gh[u]])[R] for R in range(7)] if DB & 2 else
                             _gamma(*gall(u, range(9, 13))) for u in range(NSUB)], put(dw2p), flag)
                dw_main(yS.at[2 - k], [[_ui(v) for v in gall(u, range(7))] if DB & 1 else
                                       _gamma(*gall(u, range(13, 17))) for u in range(NSUB)], put(dw1p), flag,
                        prep_pre(w2T, cn, sl[1], aB, tB, False))
                dw_put(dw2p, c, k == 1, 2 * DK, dw_tail(gS, 64, gh))
                d1 = dw_put(dw1p, c, k == 1, 2 * DK, dw_tail(yS.at[2 - k], 80, gd))
                db1_ref[:, pl.ds(pl.multiple_of(c * TF, TF), TF)] = d1[D - 2 * DK:D - 2 * DK + 1].astype(bf16)

            @pl.when(k == 2)
            def _():
                out1(c).start()
                out2(c).start()
            return sl[1], sl[2], sl[0]
        lax.fori_loop(0, NC, body, (jnp.int32(0), jnp.int32(1), jnp.int32(2)))

    def c_io(dst, t):
        return cp(io.at[t], dst.at[0, :, tok(t)], 0)

    def bwd_a(l):
        dWp[...] = jnp.zeros_like(dWp)

        def s1a(j, t):
            dy = comb(ad, j, t)
            st2(xs.at[t], j, dy)
            return dy, dy * ld2(yr.at[l, t], j).astype(f32)

        def s1b(j, t, m1, m2):
            h, o = 2 * (j // 3), R1 * (j % 3)
            base = jnp.where(l == 1, ld1(io.at[t], j).astype(f32),
                             jnp.concatenate([ax[t, h, o:o + R1, :], ax[t, h + 1, o:o + R1, :]], axis=1))
            dx = base + st[l, t, 1:2, :] * (ld1(xs.at[t], j) - m1 - ld1(yr.at[l, t], j).astype(f32) * m2)
            _st(xs.at[t], R1 * j, dx)
            _st(dxs.at[t % 2], R1 * j, dx)
            return dx

        def body(t, carry):
            flag = t < 0
            tn = nxt(t)
            pqn = lambda r0, r1: _ld(qk.at[l, t], D + r0, D + r1)
            dxb = lambda r0, r1: _ld(dxs.at[t % 2], r0, r1)
            s1, s2, dpqn, prod = [], [], [], []
            for j in range(CH):
                d = _nn(ld1(Wp.at[l], j), dxb(0, D))
                if j < 3:
                    (a0, b0), (a1_, b1) = s1a(2 * j, tn), s1a(2 * j + 1, tn)
                    g = [a0 + a1_, b0 + b1]
                    s1.append(_csum(g[0]))
                    s2.append(_csum(g[1]))
                else:
                    if j == 3:
                        m1, m2 = _cmean(sum(s1)), _cmean(sum(s2)) * (1.0 + LN_EPS)
                    g = [s1b(2 * j - 6, tn, m1, m2), s1b(2 * j - 5, tn, m1, m2)]
                dpqn.append(_gate(flag, d, g, RA))
                prod.append((dpqn[j] * pqn(R1 * j, R1 * (j + 1)).astype(f32)).astype(bf16))

            def out(j):
                v = comb(ax, j, t)
                st2(io.at[t], j, v)
                return v

            def dq(j):
                R = _head_rows(lambda h: rr[l, t, h:h + 1, :], R1 * j, R1 * (j + 1))
                a = jnp.minimum(pqn(R1 * j, R1 * (j + 1)).astype(f32) - PHI_EPS * R, R)
                C = _head_rows(lambda h: c[h:h + 1], R1 * j, R1 * (j + 1))
                v = a * (dpqn[j] - C * jnp.tile(ld1(zcol.at[l], j), (1, TS // 128)))
                _st(qk.at[l, t], R1 * j, v)
                return v
            dWp[0:R1, 0:512] += _gate(flag, _nt(pqn(0, R1), dxb(0, 512)), [out(0), out(1), out(2)], RA)
            c = _nn(_ld(hs, 0, H), jnp.concatenate(prod, axis=0))
            dxc = jnp.concatenate([dxb(512, D), *_split(c)], axis=0)
            dWp[R1:2 * R1, 0:512] += _gate(flag, _nt(pqn(R1, 2 * R1), dxb(0, 512)), [out(3), out(4), out(5)], RA)
            for j, js in ((2, [0]), (-1, [1]), (3, [2]), (4, [3, 4]), (5, [5])):
                if j < 0:
                    dWp[0:2 * R1, 512:640] += _gate(flag, _nt(pqn(0, 2 * R1), dxc), [dq(i) for i in js], RA)
                else:
                    dWp[R1 * j:R1 * (j + 1), :] += _gate(
                        flag, _nt(pqn(R1 * j, R1 * (j + 1)), jnp.concatenate([dxb(0, 512), dxc], axis=0)),
                        [dq(i) for i in js], RA)

            @pl.when(l == 1)
            def _():
                c_io(out_hbm, t).start()
            return carry
        p = [s1a(j, 0) for j in range(CH)]
        m1, m2 = _cmean(_csum(sum(a for a, _ in p))), _cmean(_csum(sum(b for _, b in p))) * (1.0 + LN_EPS)
        for j in range(CH):
            s1b(j, 0, m1, m2)
        lax.fori_loop(0, NTB, body, 0)

    def mid_bwd(l):
        dw = dWp[:, 0:D].astype(bf16)
        gb = GT[l][:, 0:D].astype(bf16)
        lane = lax.broadcasted_iota(jnp.int32, (D, 128), 1)
        hrow = lax.broadcasted_iota(jnp.int32, (D, 128), 0) // DH
        own = (lane == hrow + 64) | (lane == hrow + 96)
        dz = -jnp.sum(jnp.where(own, dWp[:, 512:640], 0.0), axis=1, keepdims=True)
        zhi, zlo = _split(dz)
        lane = lax.broadcasted_iota(jnp.int32, (D, DP - D), 1)
        zc = jnp.where(lane == 0, zhi.astype(f32), jnp.where(lane == 1, zlo.astype(f32), 0.0))
        win = [(_win(g), GR * g - _win(g)) for g in range(NG)]
        dkv = [jnp.where(masks[g % 2], _nt(dw[w:w + GW], wo[w:w + GW, :]), 0.0) for g, (w, o) in enumerate(win)]
        rows = [_nn(dkv[g][o:o + GR].astype(bf16), _ld(wqkvT, 2 * D + w, 2 * D + w + GW)) for g, (w, o) in enumerate(win)]
        a = jnp.concatenate(rows, axis=0)
        _st(a1, 0, jnp.concatenate([a, zc], axis=1))
        _st(wdu, 0, a.astype(bf16).T, slice(2 * D, 3 * D))
        for g, (w, o) in enumerate(win):
            dwo_a[GR * g:GR * (g + 1), :] += _nn(kvT[l, g], dw[w:w + GW])
        for g, (w, o) in enumerate(win):
            dwvT[GR * g:GR * (g + 1), :] += _nn(dkv[g].T[o:o + GR].astype(bf16), gb[w:w + GW])

    def bwd_b(l):
        def body(t, carry):
            flag = t < 0
            Q = lambda r0, r1: _ld(qk.at[l, t], r0, r1)
            U = lambda r0, r1: _ld(uT.at[l, t], r0, r1)
            for j in range(CH):
                dpk = _nn(ld1(a1, j), U(0, DP))
                zero_ad(flag, dpk, j, t)
                _st(qk.at[l, t], D + R1 * j, dpk * jnp.minimum(ld1(qk.at[l, t], j, 2 * D).astype(f32) - PHI_EPS, 1.0))
            r = st[l, t, 0:1, :]
            s1, s2 = [], []
            for j in range(CH):
                du = sum(_nn(ld1(wdu, j, 0, slice(a, b)), Q(a, b)) for a, b in ((2 * D, 3 * D), (0, 512), (512, 2 * D)))
                if j < 5:
                    du = _gate(flag, du, beta_io(prv(t, 2), j, t < 2), 8)
                xs[t, R1 * j:R1 * (j + 1), :] += r * du
                s1.append(_csum(du))
                s2.append(_csum(du * U(R1 * j, R1 * (j + 1)).astype(f32)))
            m1, m2 = r * _cmean(sum(s1)), r * _cmean(sum(s2))
            for j in range(CH):
                dx = ld1(xs.at[t], j) - m1 - U(R1 * j, R1 * (j + 1)).astype(f32) * m2
                _st(xs.at[t], R1 * j, dx)
                _st(io.at[t], R1 * j, dx)
                h, o = 2 * (j // 3), R1 * (j % 3)
                ax[t, h, o:o + R1, :] = dx[:, 0:P]
                ax[t, h + 1, o:o + R1, :] = dx[:, P:TS]
                dwqk[R1 * j:R1 * (j + 1), :] += _gate(flag, _nt(U(R1 * j, R1 * (j + 1)), Q(0, 2 * D)), [dx], 8)

            @pl.when(l == 0)
            def _():
                c_io(dx_hbm, t).start()
            return carry
        lax.fori_loop(0, NTB, body, 0)

        @pl.when(l == 1)
        def _():
            for tq in (NTB - 2, NTB - 1):
                for i in range(5):
                    beta_io(tq, i)

    c_dwo = cp(wo, dwo_hbm, 2)
    wv = [stg(j, 2 * D + TF * j, min(TF, D - TF * j)) for j in range(3)]
    c_dwv = [cp(buf, dwqkv_hbm.at[:, cols], 5) for buf, cols in wv]

    def stage(k, carry):
        @pl.when(k < 2)
        def _():
            fwd_a(k)

            @pl.when(k == 0)
            def _():
                for c in c_g:
                    c.start()
                c_wo.wait()
            mid_fwd(k)
            fwd_b(k)

        @pl.when(k == 0)
        def _():
            for c in c_w(0):
                c.wait()
            for c in c_w(1):
                c.start()
            prep_pre(w1, 0, 0, aF, tF, True)
            prep_pre(w2T, 0, 0, aB, tB, False)
            for c in c_g:
                c.wait()
        mlp(k)

        @pl.when(k > 0)
        def _():
            l = 2 - k
            bwd_a(l)
            mid_bwd(l)

            @pl.when(k == 1)
            def _():
                for t in range(NTB):
                    c_io(out_hbm, t).wait()

            @pl.when(k == 2)
            def _():
                wo[...] = dwo_a[...].astype(bf16)
                c_dwo.start()
                for c in range(NC):
                    out1(c).wait()
                for j, (buf, _) in enumerate(wv):
                    buf[...] = dwvT[TF * j:TF * j + buf.shape[1], :].astype(bf16).T
                    c_dwv[j].start()
                ones = jnp.ones((16, 128), bf16)
                hi = _b16(db2a[...])
                db2_ref[...] = (_nt(ones, hi) + _nt(ones, _b16(db2a[...] - _ui(hi))))[0:1].astype(bf16)
            bwd_b(l)
        return carry
    lax.fori_loop(0, 3, stage, 0)

    c_dwq = []
    for j in range(5):
        buf, cols = stg(3 + j, TF * j, min(TF, 2 * D - TF * j))
        buf[...] = dwqk[:, cols].astype(bf16)
        c_dwq.append(cp(buf, dwqkv_hbm.at[:, cols], 1))
        c_dwq[-1].start()
    for c in c_w(1) + [c_dwo] + c_dwv:
        c.wait()
    for c in range(NC):
        out2(c).wait()
    for t in range(NTB):
        c_io(dx_hbm, t).wait()
    for c in c_dwq:
        c.wait()


@jax.jit
def pallas_interleave_layers__linear_attn_block__mixer_channel_mlp__prompt_kernel(A_x, A_wqkv, A_wo, B_x, B_w1, B_b1, B_w2, B_b2, grad_out):
    anyspec = pl.BlockSpec(memory_space=pl.ANY)
    vspec = pl.BlockSpec(memory_space=pltpu.VMEM)
    V = pltpu.VMEM

    def PB(*s):
        return V(s[:-2] + (s[-2] // 2, s[-1]), u32) if PK else V(s, bf16)
    scratch = [
        V((NTB, D, TS), bf16),
        V((D, 64), bf16),
        PB(D, 3 * D),
        PB(3 * D, D),
        V((D, D), bf16),
        V((3, D, TF), bf16),
        V((3, D, TF), bf16),
        V((NTB, D, TS), f32),
        V((NTB, 7, DM, P), f32),
        V((NTB, 7, DM, P), f32),
        PB(NTB, BT + 128, P),
        PB(2, D, TS),
        PB(2, NTB, DP, TS),
        PB(2, NTB, 3 * D, TS),
        PB(2, NTB, BT + 160, P),
        PB(2, NTB, D, TS),
        PB(NC + 1, 4, NSUB, HF, SW),
        V((NC, DP, TF), bf16),
        V((NC, D, TF), bf16),
        PB(49, 64, 128),
        PB(TF, 80),
        PB(49, 64, 128),
        PB(TF, 64),
        V((2, NTB, 8, TS), f32),
        V((2, NTB, H, TS), f32),
        V((2, D, DP), f32),
        PB(2, D, D),
        PB(D, D),
        V((2, NG, GR, GW), bf16),
        PB(H, D),
        PB(H, D),
        V((2, D, 128), f32),
        V((D, 640), f32),
        V((D, 2 * D), f32),
        V((D, D), f32),
        V((D, D), f32),
        PB(D, DP),
        V((D, 128), f32),
        V((D, 128), f32),
        pltpu.SemaphoreType.DMA((7,)),
    ]
    sds = jax.ShapeDtypeStruct
    outs = pl.pallas_call(
        _kernel,
        in_specs=[anyspec, anyspec, anyspec, anyspec, vspec, anyspec, vspec, anyspec],
        out_specs=[anyspec, anyspec, anyspec, anyspec, anyspec, vspec, anyspec, vspec],
        out_shape=[sds((1, D, S), bf16), sds((1, D, S), bf16), sds((D, 3 * D), bf16), sds((D, D), bf16),
                   sds((D, F), bf16), sds((1, F), bf16), sds((D, F), bf16), sds((1, D), bf16)],
        scratch_shapes=scratch,
        compiler_params=pltpu.CompilerParams(vmem_limit_bytes=128 * 1024 * 1024 - 128 * 1024,
                                             disable_bounds_checks=True),
    )(jnp.swapaxes(A_x, 1, 2), A_wqkv, A_wo, B_w1, B_b1.reshape(1, F), B_w2.T, B_b2.reshape(1, D),
      jnp.swapaxes(grad_out, 1, 2))
    out, dx, dwqkv, dwo, dw1, db1, dw2, db2 = outs
    return (jnp.swapaxes(out, 1, 2), jnp.swapaxes(dx, 1, 2), dwqkv, dwo, dw1, db1.reshape(F), dw2.T,
            db2.reshape(D))
```

```python
import jax
import jax.numpy as jnp
from jax import lax
import jax.experimental.pallas as pl
import jax.experimental.pallas.tpu as pltpu

S, D, F = 2048, 576, 4608
H, DH = 32, 18
DP = 592
NG, GR, GW = 8, 72, 80
TS = 256
P = TS // 2
NTB = S // TS
TF = 256
HF = TF // 2
NC = F // TF
NSUB = 4
BS = NTB // NSUB
SW = BS * P
DK, DM = 256, 288
LN_EPS = 1e-5
PHI_EPS = 1e-6
C0 = 0.7978845608028654
C1 = 0.044715 * C0
bf16, f32, u32 = jnp.bfloat16, jnp.float32, jnp.uint32
CH = 6
R1, RA = D // CH, DM // CH
QCH = [(0, 128), (128, 256), (256, 384), (384, 512), (512, 576)]
ALL = slice(None)
PK = True


def _nn(a, b):
    return jnp.dot(a, b, preferred_element_type=f32)


def _nt(a, b):
    return lax.dot_general(a, b, (((1,), (1,)), ((), ())), preferred_element_type=f32)


def _rows(ref, r0, n, z):
    k = 2 if ref.dtype == u32 else 1
    if isinstance(z, int):
        r0, z = r0 + 64 * z, None
    if z is None:
        return slice(r0 // k, (r0 + n) // k)
    return pl.ds(pl.multiple_of(r0 // k + z * (64 // k), 16 // k), n // k)


def _ld(ref, r0, r1, cols=ALL, z=None):
    v = ref[_rows(ref, r0, r1 - r0, z), cols]
    return pltpu.bitcast(v, bf16) if ref.dtype == u32 else v


def _up(w):
    return w if w.dtype == f32 else pltpu.bitcast(w, bf16).astype(f32)


def _st(ref, r0, v, cols=ALL, z=None):
    if ref.dtype == u32:
        w = v if v.dtype == u32 else pltpu.bitcast(v.astype(bf16), u32)
        rows = _rows(ref, r0, 2 * w.shape[0], z)
        ref[rows, cols] = w
        return lax.bitcast_convert_type(ref[rows, cols], f32)
    ref[_rows(ref, r0, v.shape[0], z), cols] = v.astype(ref.dtype)
    return v


def _half(n):
    return slice(128 * (n % 2), 128 * (n % 2 + 1))


def _win(g):
    return GR * g - 8 * (g % 2)


def _split(a):
    hi = a.astype(bf16)
    lo = (a - hi.astype(f32)).astype(bf16)
    return hi, lo


def _csum(x):
    return x.reshape(x.shape[0] // 8, 8, x.shape[1]).sum(axis=0)


def _cmean(s):
    return jnp.sum(s, axis=0, keepdims=True) * (1.0 / D)


def _head_rows(row, r0, r1):
    b = {}

    def get(h):
        if h not in b:
            v = row(h)
            b[h] = jnp.broadcast_to(v, (8, v.shape[1]))
        return b[h]
    rows = []
    for j in range(r0 // 8, r1 // 8):
        h0, h1 = (8 * j) // DH, (8 * j + 7) // DH
        if h0 == h1:
            rows.append(get(h0))
        else:
            sub = lax.broadcasted_iota(jnp.int32, get(h0).shape, 0)
            rows.append(jnp.where(sub < h1 * DH - 8 * j, get(h0), get(h1)))
    return jnp.concatenate(rows, axis=0)


def _gate(flag, d, vals, br, spread=False):
    nr, nc = d.shape[0] // br, d.shape[1] // 128
    blk = [d[br * i:br * (i + 1), 128 * j:128 * (j + 1)] for i in range(nr) for j in range(nc)]
    vs = [v[br * i:br * (i + 1), 128 * j:128 * (j + 1)]
          for v in vals for i in range(v.shape[0] // br) for j in range(v.shape[1] // 128)]
    for n, v in enumerate(vs):
        m = n * len(blk) // len(vs) if spread else n % len(blk)
        blk[m] = jnp.where(flag, v, blk[m])
    out = jnp.concatenate([jnp.concatenate(blk[nc * i:nc * (i + 1)], axis=1) for i in range(nr)], axis=0)
    if nc * 128 < d.shape[1]:
        out = jnp.concatenate([out, d[0:nr * br, nc * 128:]], axis=1)
    return out


def _gelu(x):
    x2 = x * x
    s = 0.5 * jnp.tanh(x * (C0 + C1 * x2)) + 0.5
    h = x * s
    return h, s + h * (1.0 - s) * (2.0 * C0 + 6.0 * C1 * x2)


def _quad(a11, a12, a21, a22):
    return jnp.concatenate([jnp.concatenate([a11, a12], axis=1), jnp.concatenate([a21, a22], axis=1)], axis=0)


def _alpha(a11, a12, a21, a22):
    return [a11 + a22, a21 + a22, a11, a22, a11 + a12, a21 - a11, a12 - a22]


def _beta(b11, b12, b21, b22):
    return [b11 + b22, b11, b12 - b22, b21 - b11, b22, b11 + b12, b21 + b22]


def _gamma(c11, c12, c21, c22):
    return [c11 + c22, c21 - c22, c12 + c22, c11 + c21, c12 - c11, c22, c11, c12, c21]


def _gamma_n(c11, c12, c21, c22):
    return [c11 - c22, c22 - c21, c12 - c22, c11 - c21, c11 - c12, c22, c11]


GN = ((0, 3), (3, 2), (1, 3), (0, 2), (0, 1), (3,), (0,))
GP = ((0, 3, 1), (2, 3, -1), (1, 3, 1), (0, 2, 1), (1, 0, -1), (3,), (0,))


def _gamma2(x, R, r):
    q, i = GN[R], GP[r]
    pm = lambda a, b, t: a + b if t > 0 else a - b
    if len(q) == 1:
        return x[q[0]][i[0]] if len(i) == 1 else pm(x[q[0]][i[0]], x[q[0]][i[1]], i[2])
    if len(i) == 1:
        return x[q[0]][i[0]] - x[q[1]][i[0]]
    return pm(x[q[0]][i[0]], x[q[1]][i[1]], -i[2]) - pm(x[q[1]][i[0]], x[q[0]][i[1]], -i[2])


def _beta_t(a):
    return _quad(a[0] + a[1] - a[3] + a[5], a[2] + a[5], a[3] + a[6], a[0] - a[2] + a[4] + a[6])


def _alpha_t(e):
    return _quad(e[0] + e[2] + e[4] - e[5], e[4] + e[6], e[1] + e[5], e[0] + e[1] + e[3] - e[6])


def _prod7(f, t=None):
    m2 = f(2); m4 = f(4)
    c12 = m2 + m4 if t is None else m2 + m4 + t(1)
    m1 = f(1); m3 = f(3)
    c21 = m1 + m3 if t is None else m1 + m3 + t(2)
    m0 = f(0)
    c11 = m3 - m4 + m0 + f(6)
    c11 = c11 if t is None else c11 + t(0)
    c22 = m2 - m1 + m0 + f(5)
    c22 = c22 if t is None else c22 + t(3)
    return c11, c12, c21, c22


ORD = (2, 4, 1, 3, 0, 6, 5)
DB = 0
LAG = 12
GV = 13
PA = 0
PB_ = 24
U1 = 2
U2 = 3
U3 = 1
FV = 3
FS1 = [[[], [0, 1], [2], [3], [4], [5]], [[], [0, 1, 2], [3], [4], [5], []], [[], [0, 1, 2], [3, 4], [5], [], []], [[0], [1, 2], [3], [4], [5], []]][FV]
FS3 = [[[], [4], [0], [1], [2], [3]], [[], [], [0], [1], [2], [3, 4]], [[], [], [0], [1], [2, 4], [3]], [[], [4], [0], [1], [2], [3]]][FV]
YF = 1
BV = [((2, [0], []), (-1, [1], []), (3, [2, 3], [0, 1]), (4, [4], [2, 3]), (5, [5], [4, 5])),
      ((2, [], [0, 1, 2]), (-1, [0], []), (3, [1], [3, 4, 5]), (4, [2, 3], []), (5, [4, 5], []))][0]
OF = 0
TI = 2
TR = [(5, 6), (0, 2, 3), range(7)][1]
DWG = (0, 2, 4, 5)
DWL = 4


def _w32(v):
    return lax.bitcast_convert_type(pltpu.bitcast(v, u32), f32)


def _blocks(a):
    n, m = a.shape[0] // 2, a.shape[1] // 2
    return a[0:n, 0:m], a[0:n, m:], a[n:, 0:m], a[n:, m:]


BT = 25 * 64


def _kernel(x_hbm, wqkv_hbm, wo_hbm, w1_hbm, b1_ref, w2_hbm, b2_ref, g_hbm,
            out_hbm, dx_hbm, dwqkv_hbm, dwo_hbm, dw1_hbm, db1_ref, dw2_hbm, db2_ref,
            io, wt, wdu, wqkvT, wo, w12, xsf, ax, ad, gS, dxs, uT, qa, qk, yS, yr, pre_s, dw1p, dw2p,
            aFB, tF, tB, wT, b1s,
            stf, rr, GT, Wp, WpT, kvT, zh, hs, zcol, dWp, dwqk, dwvT, dwo_a, a1, b2c, db2a, own, b1v, b2v, zs, sem):
    zs[0] = 0
    w1, w2T, aF, aB = w12.at[0], w12.at[1], aFB.at[0], aFB.at[1]
    xs, st = xsf.at[pl.ds(2, NTB)], stf.at[:, pl.ds(2, NTB)]

    def cp(src, dst, k):
        return pltpu.make_async_copy(src, dst, sem.at[k])

    def tok(t):
        return pl.ds(pl.multiple_of(t * TS, TS), TS)

    c_x = [cp(x_hbm.at[0, :, tok(t)], io.at[t], 0 if t > 2 else 5 if t else 2) for t in range(NTB)]

    def stg(j, c0, n):
        return (wt if n == 64 else dw1p.at[j, pl.ds(0, D), pl.ds(0, n)]), pl.ds(c0, n)
    wq = [stg(j, TF * j, TF) for j in range(6)] + [stg(6, 6 * TF, 128), stg(7, 6 * TF + 128, 64)]
    c_wqkv = [cp(wqkv_hbm.at[:, cols], buf, (1, 1, 1, 3, 3, 4, 4, 4)[j]) for j, (buf, cols) in enumerate(wq)]
    c_wo = cp(wo_hbm, wo, 2)

    def c_w(c, sl=None):
        cols = pl.ds(pl.multiple_of(c * TF, TF), TF)
        sl = c if sl is None else sl
        return [cp(w1_hbm.at[:, cols], w1.at[sl], 6), cp(w2_hbm.at[:, cols], w2T.at[sl], 6)]
    c_g = [cp(g_hbm.at[0, :, tok(t)], io.at[t], 5) for t in range(NTB)]
    b1v = b1v.at[pl.ds(0, F)]
    c_b = [cp(b1_ref, b1v, 7), cp(b2_ref, b2v, 7)]
    c_db = [cp(b1v, db1_ref, 7), cp(b2v, db2_ref, 7)]
    for c in c_x[0:1] + c_wqkv[0:3] + c_b + c_wqkv[3:5] + c_x[1:3] + c_wqkv[5:8] + c_x[3:]:
        c.start()

    ones_rows = (lax.broadcasted_iota(jnp.int32, (DP - D, TS), 0) < 2).astype(f32)
    one_row = (lax.broadcasted_iota(jnp.int32, (DP - D, TS), 0) < 1).astype(f32)
    for l in range(2):
        for t in range(NTB):
            _st(uT.at[l, t], D, ones_rows)
            _st(yS.at[l, t], BT + 64, one_row)
    stf[...] = jnp.zeros_like(stf)
    xsf[0:2] = jnp.zeros((2, D, TS), f32)
    rj = lax.broadcasted_iota(jnp.int32, (GW, GW), 0)
    ci = lax.broadcasted_iota(jnp.int32, (GW, GW), 1)
    masks = [rj // DH == ci // DH, (rj + (DH - 8)) // DH == (ci + (DH - 8)) // DH]
    hsel = lax.broadcasted_iota(jnp.int32, (H, D), 0) == lax.broadcasted_iota(jnp.int32, (H, D), 1) // DH
    _st(hs, 0, hsel.astype(f32))
    GT[...] = jnp.zeros_like(GT)
    lane = lax.broadcasted_iota(jnp.int32, (D, 128), 1)
    hrow = lax.broadcasted_iota(jnp.int32, (D, 128), 0) // DH
    own[...] = ((lane == hrow + 64) | (lane == hrow + 96)).astype(f32)
    dWp[...] = jnp.zeros_like(dWp)
    row0 = lax.broadcasted_iota(jnp.int32, (DP - D, TF), 0) == 0

    def wq_prep(js):
        for c in [c_wqkv[j] for j in js] + (c_b if js[0] == 0 else []):
            c.wait()
        for j in js:
            buf, cols = wq[j]
            _st(wqkvT, cols.start, buf[...].T)
            n = min(TF, 2 * D - TF * j)
            if n > 0:
                _st(wdu, 0, buf[:, 0:n], slice(TF * j, TF * j + n))
        if js[0] == 0:
            dwqk[...] = jnp.zeros_like(dwqk)
            b2c[...] = jnp.broadcast_to(b2v[...].astype(f32).reshape(1, D), (128, D)).T
            b1s[0:1] = b1v[...].astype(f32).reshape(1, F)
        if js[0] == 3:
            dwvT[...] = jnp.zeros_like(dwvT)
            dwo_a[...] = jnp.zeros_like(dwo_a)
    c_x[0].wait()

    def ld2(ref, j):
        return jnp.concatenate([_ld(ref, RA * j, RA * (j + 1)), _ld(ref, DM + RA * j, DM + RA * (j + 1))], axis=0)

    def st2(ref, j, v):
        _st(ref, RA * j, v[0:RA])
        _st(ref, DM + RA * j, v[RA:R1])

    def ld1(ref, j, o=0, cols=ALL):
        return _ld(ref, o + R1 * j, o + R1 * (j + 1), cols)

    def comb(acc, j, t, tie=None):
        a = [acc[t, r, RA * j:RA * (j + 1), :] for r in range(7)]
        if tie is not None:
            a = [jnp.where(zs[0] > 0, _blocks(tie)[r % 4], v) if r in TR else v for r, v in enumerate(a)]
        return _beta_t(a)

    def put_beta(dst, get, tq, z, i, colsum=False):
        if i == 4:
            w = get(tq, z, 2 * DK, 64, None)
            g = [_st(dst.at[tq], BT, w)]
            if colsum:
                v = _up(w)
                g.append(_st(db2a, 2 * DK, db2a[2 * DK:D] + (v[:, 0:P] + v[:, P:TS])))
            return g
        v = [[[_up(get(tq - z + j, j, DK * K + 128 * k + 16 * i, 16, z)) for j in range(2)] for k in range(2)] for K in range(2)]
        b1 = [[_beta(v[0][k][j][:, 0:P], v[0][k][j][:, P:TS], v[1][k][j][:, 0:P], v[1][k][j][:, P:TS])
               for j in range(2)] for k in range(2)]
        g = []
        for R in range(7):
            b2 = _beta(b1[0][0][R], b1[0][1][R], b1[1][0][R], b1[1][1][R])
            w32 = [_st(dst.at[tq], 64 * ((7 * R + r) // 2) + 16 * i, b2[r], _half(7 * R + r)) for r in range(7)]
            g += [w32, b2, [b[8 * (r % 2):8 * (r % 2 + 1)] for r, b in enumerate(b2)]][U2 - 2]
            if colsum and R >= 5:
                for k in range(2):
                    o = DK * (R - 5) + 128 * k + 16 * i
                    g.append(_st(db2a, o, _ld(db2a, o, o + 16, z=z) + b2[5 + k], z=z))
        return g

    def beta_io(tq, z, i, skip=None):
        def get(tb, j, a, n, z):
            w = pltpu.bitcast(_ld(io.at[tb], a, a + n, z=z), u32)
            return w if skip is None else jnp.where(skip, jnp.uint32(0), w)
        return put_beta(gS, get, tq, z, i, True)

    def zero_ad(flag, d, j, t, acc=ad, rs=range(7)):
        z = [jnp.where(flag, d[RA * a:RA * (a + 1), P * b:P * (b + 1)], 0.0) for a in range(2) for b in range(2)]
        for r in rs:
            acc[t, r, RA * j:RA * (j + 1), :] = z[r % 4]

    def phi(z):
        return (jnp.where(z > 0, z + 1.0, jnp.exp(z)) + PHI_EPS).astype(bf16)

    pair = lambda body: lambda t2, c: body(2 * t2 + 1, 1, body(2 * t2, 0, c))
    nxt = lambda t, n=1: jnp.minimum(t + n, NTB - 1)
    prv = lambda t, n=1: jnp.maximum(t - n, 0)

    def fwd_a(l):
        db2a[...] = jnp.zeros_like(db2a)

        def s1a(j, t):
            x = jnp.where(l == 0, ld2(io.at[t], j).astype(f32), comb(ax, j, t))
            st2(xs.at[t], j, x)
            return x

        def s1b(j, t, m):
            xc = ld1(xs.at[t], j) - m
            return xc * xc

        def s1r(t, sv):
            r = lax.rsqrt(_cmean(sv) + LN_EPS)
            st[l, t, 0:1, :] = r
            return r

        def s1c(r0, r1, t, m, r):
            u = (xs[t, r0:r1, :] - m) * r
            return _st(uT.at[l, t], r0, u)

        def body2(t2, carry):
            @pl.when((l == 0) & (t2 == 1))
            def _():
                for c in c_x[3:]:
                    c.wait()
                for c in [c_wo] + c_w(0):
                    c.start()
                wq_prep((5, 6, 7))
            return pair(body)(t2, carry)

        def body(t, z, carry):
            flag = zs[0] > 0 if OF & 1 else t < 0
            tn = nxt(t)
            ub = _ld(uT.at[l, t], 0, D)
            sm = []
            for j in range(CH):
                x = s1a(j, tn)
                sm.append(_csum(x))
                k = _nn(ld1(wqkvT, j, D), ub)
                zero_ad(flag, k, j, t)
                _st(qk.at[l, t], D + R1 * j, phi(_gate(flag, k, [x], RA)))
            m = _cmean(sum(sm))
            sv = []
            for j in range(CH):
                sq = s1b(j, tn, m)
                sv.append(_csum(sq))
                q = _nn(ld1(wqkvT, j), ub)
                _st(qa.at[t], R1 * j, phi(_gate(flag, q, [sq], RA)))
            r = s1r(tn, sum(sv))
            for j, (r0, r1) in enumerate(QCH):
                d = _nt(_ld(qk.at[l, t], D + r0, D + r1), _ld(uT.at[l, t], 0, DP))
                u = s1c(r0, r1, tn, m, r)
                b = beta_io(t, z, j)
                GT[l, r0:r1, :] += _gate(flag, d, [u] + b, 8)
            return carry
        m = _cmean(sum([_csum(s1a(j, 0)) for j in range(CH)]))
        r = s1r(0, sum([_csum(s1b(j, 0, m)) for j in range(CH)]))
        s1c(0, D, 0, m, r)

        @pl.when(l == 0)
        def _():
            wq_prep((0, 1, 2))
            wq_prep((3, 4))
            for c in c_x[1:3]:
                c.wait()
        lax.fori_loop(0, NTB // 2, body2, 0)

    def mid_fwd(l):
        zcol[l] = jnp.broadcast_to(GT[l, :, D:D + 1], (D, 128))
        sel = (lax.broadcasted_iota(jnp.int32, (H, DP - 512), 1) == D - 512).astype(f32).astype(bf16)
        _st(zh, 0, jnp.where(hsel, _nt(sel, GT[l, :, 512:DP].astype(bf16)), 0.0))
        win = [(_win(g), GR * g - _win(g)) for g in range(NG)]
        kv = [jnp.where(masks[g % 2], _nt(GT[l, w:w + GW, 0:D].astype(bf16), _ld(wqkvT, 2 * D + w, 2 * D + w + GW)), 0.0)
              for g, (w, o) in enumerate(win)]
        rows = [_nn(kv[g][o:o + GR].astype(bf16), wo[w:w + GW, :]) for g, (w, o) in enumerate(win)]
        for g, (w, o) in enumerate(win):
            kvT[l, g] = kv[g].T[o:o + GR].astype(bf16)
        wp = jnp.concatenate(rows, axis=0).astype(bf16)
        _st(Wp.at[l], 0, wp)
        _st(WpT, 0, wp.T)

    def fwd_b(l):
        def den(t, r):
            r[...] = 1.0 / (_nn(_ld(zh, 0, H), _ld(qa.at[t], 0, D)) + PHI_EPS)

        def s1(j, t, r, q):
            v = ld1(qa.at[t], j).astype(f32) * _head_rows(lambda h: r[h:h + 1, :], R1 * j, R1 * (j + 1))
            w = _st(q, R1 * j, v)
            return v if YF == 2 else w

        def s3r(x, s, m):
            sq = [m - ld1(x, j) for j in range(CH)]
            sq = sum(v * v for v in sq)
            s[1:2, :] = lax.rsqrt(_cmean(_csum(sq)) * (1.0 + LN_EPS) + LN_EPS * LN_EPS)
            s[2:3, :] = m
            return sq

        def s3b(i, tq, z0, xv, sv):
            def get(tb, j, a, n, z):
                y = (_ld(xv.at[j], a, a + n, z=z) - sv[j, 2:3, :]) * sv[j, 1:2, :]
                w = lax.bitcast_convert_type(_st(yr.at[l, tb], a, y, z=z), u32)
                return y if n == 16 else w
            return put_beta(yS.at[l], get, tq, z0, i)

        def body(t2, sm):
            xv, sv = xsf.at[pl.ds(2 * t2, 4)], stf.at[l, pl.ds(2 * t2, 4)]
            qv, rv = qk.at[l, pl.ds(2 * t2, 3)], rr.at[l, pl.ds(2 * t2, 4)]
            flag = zs[0] > 0
            for z in range(2):
                t = 2 * t2 + z
                ns = []
                for j in range(CH):
                    d = _nn(ld2(WpT, j), _ld(qv.at[z], 0, D))
                    g = [s1(i, nxt(t), rv.at[z + 1], qv.at[z + 1]) for i in FS1[j]]
                    if j == 0:
                        g.append(s3r(xsf.at[t + 1 + zs[0]] if U3 == 2 else xv.at[z + 1], sv.at[z + 1], _cmean(sm)))
                    for i in FS3[j]:
                        g += s3b(i, jnp.maximum(t - 2, z), z, xv, sv)
                    x = ld2(xv.at[z + 2], j) + _gate(flag, d, g, 8)
                    st2(xv.at[z + 2], j, x)
                    ns.append(_csum(x))
                    xb = x + jnp.tile(ld2(b2c, j), (1, TS // 128))
                    x11, x12, x21, x22 = xb[0:RA, 0:P], xb[0:RA, P:TS], xb[RA:R1, 0:P], xb[RA:R1, P:TS]
                    zero = jnp.where(flag, x11, 0.0)
                    for r, val in enumerate([zero, x11 + x21, x12, x21, x22 + x12, zero, zero]):
                        ax[t, r, RA * j:RA * (j + 1), :] = val
                    if j == 0:
                        den(nxt(t, 2), rv.at[z + 2])
                sm = sum(ns)
            return sm
        den(0, rr.at[l, 0])
        den(1, rr.at[l, 1])
        for j in range(CH):
            s1(j, 0, rr.at[l, 0], qk.at[l, 0])
        m = _cmean(lax.fori_loop(0, NTB // 2, body, jnp.zeros((8, TS), f32)))
        s3r(xs.at[NTB - 1], st.at[l, NTB - 1], m)
        for tq in (NTB - 2, NTB - 1):
            for i in range(5):
                s3b(i, tq, tq % 2, xsf.at[pl.ds(NTB, 2)], stf.at[l, pl.ds(NTB, 2)])

    def prep_t(w, sl):
        _st(wT, 0, w[sl, 0:2 * DK, :].T)

    def prep_pre(w, c, sl, dst, tail, bias, flag=None):
        g = []
        for R in range(7):
            z = None if flag is None else jnp.where(flag, R + 1, 0)
            a = _alpha(*[_ld(wT, HF * i, HF * (i + 1), slice(DK * j, DK * (j + 1)), z).astype(f32)
                         for i in range(2) for j in range(2)])
            al = _alpha(*_blocks(a[R]))
            w32 = [_st(dst.at[(7 * R + r) // 2], 0, al[r], _half(7 * R + r)) for r in range(7)]
            g += al if GV & 1 else w32
        if tail is not None:
            prep_tail(w, c, sl, tail, bias)
        return g

    def prep_tail(w, c, sl, tail, bias):
        tl = w[sl, 2 * DK:D, :]
        if bias:
            b = b1s[0:1, pl.ds(pl.multiple_of(c * TF, TF), TF)]
            tl = jnp.concatenate([tl, jnp.where(row0, jnp.broadcast_to(b, (DP - D, TF)), 0.0).astype(bf16)], axis=0)
        _st(tail, 0, tl.T)

    def prep_dy(w, sl):
        W = lambda r, q: w[sl, DM * r:DM * (r + 1), HF * q:HF * (q + 1)].astype(f32)
        return [v.astype(bf16) for v in _alpha(W(0, 0), W(1, 0), W(0, 1), W(1, 1))]

    def bop(bS, p, n):
        return jnp.concatenate([_ld(bS.at[2 * p + z], 64 * (n // 2), 64 * (n // 2 + 1), _half(n)) for z in range(2)], axis=0)

    def btail(bS, T, p, J):
        return jnp.concatenate([_ld(bS.at[2 * p + j], BT, BT + T, _half(J)) for j in range(2)], axis=1)

    hist = []

    def prelike(a, tail, bS, T, p, flag=None, work=None, pre=None):
        def M(R):
            i = ORD.index(R)
            if pre is not None:
                pre(i)

            def f(r):
                d = _nn(_ld(a.at[(7 * R + r) // 2], 0, 64, _half(7 * R + r)), bop(bS, p, 7 * R + r))
                g = work(7 * i + ORD.index(r)) if work is not None else []
                hist.append(d[0:8])
                return _gate(flag, d, g, 8) if g else d
            return _quad(*_prod7(f))
        return _prod7(M, lambda q: _nn(_ld(tail, HF * (q // 2), HF * (q // 2 + 1)), btail(bS, T, p, q % 2)))

    def dy1(b, ga, acc, u, r, flag=None, g=()):
        d = _nn(b[r], ga[r])
        hist.extend([d[96 * i:96 * i + 8, 0:128] for i in range(3)])
        if len(g):
            d = _gate(flag, d, g, 8, True)
        for i in range(BS):
            acc[BS * u + i, r] += d[:, P * i:P * (i + 1)]
        return d

    def dylike(b, ga, acc, u, gate=None):
        for r in range(7):
            dy1(b, ga, acc, u, r, *(() if gate is None else (gate[0], gate[1][7 * r:7 * (r + 1)])))

    def dw_main(bS, g1, put, flag, gate=None):
        E, pend = {}, []
        for m, R in enumerate((4, 6, 1, 5, 0, 2, 3)):
            if GV & 8:
                ops = [[_gamma2([_blocks(v) for v in g], R, r) for r in range(7)] for g in g1]
            else:
                ops = [_gamma(*_blocks(_gamma_n(*g)[R]))[0:7] for g in g1]
            e = []
            for r in range(7):
                n = 7 * R + r
                d = _nt(jnp.concatenate([o[r] for o in ops], axis=1).astype(bf16),
                        jnp.concatenate([bop(bS, p, n) for p in range(NSUB)], axis=1))
                g = [] if gate is None else [gate[7 * m + r]]
                if r >= 3 and pend:
                    g.append(pend[0][64 * (r - 3):64 * (r - 2)])
                e.append(_gate(flag, d, g, 8) if g else d)
            E[R] = _alpha_t(e)
            pend = []
            if R == 6:
                pend = [put(1, 0, (E[6] - E[4] if GV & 4 else E[4] + E[6]).T)]
            if R == 5:
                pend = [put(0, 1, (E[5] - E[1] if GV & 4 else E[1] + E[5]).T)]
            if R == 2:
                pend = [put(0, 0, (E[0] + E[2] - E[4] + E[5] if GV & 4 else E[0] + E[2] + E[4] - E[5]).T)]
            if R == 3:
                put(1, 1, (E[6] - E[0] - E[1] - E[3] if GV & 4 else E[0] + E[1] + E[3] - E[6]).T)

    def dw_tail(bS, T, gs, flag=None, gate=None):
        if gate is None:
            return _nt(jnp.concatenate([btail(bS, T, p, J) for p in range(NSUB) for J in range(2)], axis=1),
                       jnp.concatenate([_quad(*g) for g in gs], axis=1).astype(bf16))
        n = len(gate)
        return sum(_gate(flag, _nt(btail(bS, T, p, J), jnp.concatenate(gs[p][J::2], axis=0).astype(bf16)),
                         gate[n * (2 * p + J) // 8:n * (2 * p + J + 1) // 8], 8)
                   for p in range(NSUB) for J in range(2))

    def dw_put(dst, c, first, r0, v, c0=0):
        idx = (c, slice(r0, r0 + v.shape[0]), slice(c0, c0 + v.shape[1]))
        tot = jnp.where(first, 0.0, dst[idx].astype(f32)) + v
        dst[idx] = tot.astype(bf16)
        return tot

    def out1(c):
        return cp(dw1p.at[c, pl.ds(0, D), :], dw1_hbm.at[:, pl.ds(pl.multiple_of(c * TF, TF), TF)], 3)

    def out2(c):
        return cp(dw2p.at[c], dw2_hbm.at[:, pl.ds(pl.multiple_of(c * TF, TF), TF)], 4)

    def mlp(k):
        def body(c, sl):
            cn = jnp.where(c + 1 < NC, c + 1, 0)
            ps = jnp.where(k == 1, NC, c)
            flag = c < 0

            def pres(q, u, n, t=None):
                w = pre_s[ps, q, u, 8 * (n // 2):8 * (n // 2 + 1), P * (n % 2):P * (n % 2 + 1)]
                if t is not None:
                    w = jnp.where(flag, t, w)
                return _up(w)

            def cat(G, u, rs):
                return [jnp.concatenate([jnp.concatenate([G[u, 2 * i + j][r] for j in range(2)], axis=1)
                                         for i in range(8)], axis=0) for r in rs]
            for d in c_w(cn, sl[1]):
                d.wait()
            for d in c_w(jnp.where(c + 2 < NC, c + 2, c + 2 - NC), sl[2]):
                d.start()

            @pl.when(k < 2)
            def _():
                pre, G = {}, {}
                b = prep_dy(w2T, sl[0])
                prep_t(w1, sl[1])

                def piece(u, n):
                    G[u, n] = [_gelu(pres(q, u, n))[0] for q in range(4)]
                    return G[u, n]

                def gall(u):
                    return [v.astype(bf16) for v in _gamma(*cat(G, u, range(4)))[0:7]]
                for s in range(NSUB + 2):
                    ga = gall(s - 2) if s >= 2 else None
                    if s < NSUB:
                        pre[s] = prelike(aF, tF, yS.at[k], 80, s, flag,
                                         (lambda n: piece(s - 1, n // 3) if n % 3 == 2 else []) if s >= 1 else None,
                                         (lambda i: dy1(b, ga, ax, s - 2, i)) if s >= 2 else None)
                        for q in range(4):
                            _st(pre_s.at[ps, q, s], 0, pre[s][q])
                    elif s == NSUB:
                        for r in range(7):
                            dy1(b, ga, ax, s - 2, r, flag,
                                [v for n in range(16 * r // 7, 16 * (r + 1) // 7) for v in piece(s - 1, n)])
                    else:
                        dylike(b, ga, ax, s - 2, (flag, prep_pre(w1, cn, sl[1], aF, tF, True, flag)))

            @pl.when(k > 0)
            def _():
                dh, G, HG = {}, {}, {}
                b = prep_dy(w1, sl[0])
                prep_t(w2T, sl[1])

                def pa(u, n, t=None):
                    HG[u, n] = [_gelu(pres(q, u, n, t)) for q in range(4)]
                    return [g for _, g in HG[u, n]]

                def pb(u, n):
                    i, j = n // 2, n % 2
                    if (u, n) not in HG:
                        pa(u, n)
                    dp = [d[16 * i:16 * (i + 1), P * j:P * (j + 1)] * g for d, (_, g) in zip(dh[u], HG[u, n])]
                    G[u, n] = [a for a, _ in HG[u, n]] + dp
                    return dp

                def gall(u, rs):
                    return cat(G, u, rs)
                jobs = [[(pa, 0, n) for n in range(0, 16, 2)]] + [[(pb, u, n) for n in range(16)] for u in range(NSUB)]
                dys = [[], [], [(0, r) for r in range(4)], [(0, 4), (0, 5), (0, 6), (1, 0)],
                       [(1, r) for r in range(1, 7)] + [(2, r) for r in range(7)]]

                def work(s, n, tot):
                    J = jobs[s]
                    return [v for f, u, i in J[len(J) * n // tot:len(J) * (n + 1) // tot] for v in f(u, i)]

                def dy(u, r, g=()):
                    c = gall(u, range(4, 8))
                    if GV & 2:
                        c[0], c[3] = jnp.where(flag, 0.0, c[0]), jnp.where(flag, 0.0, c[3])
                    dy1(b, {r: _gamma(*c)[r].astype(bf16)}, ad, u, r, flag, g)
                for s in range(NSUB + 1):
                    if s < NSUB:
                        dh[s] = prelike(aB, tB, gS, 64, s, flag, lambda n: work(s, n, 49),
                                        lambda i: [dy(*x) for x in dys[s][i // 2:i // 2 + 1]] if i % 2 == 0 else None)
                    else:
                        for m, x in enumerate(dys[s]):
                            dy(*x, work(s, m, len(dys[s])))
                gh = [gall(u, range(4)) for u in range(NSUB)]
                gd = [gall(u, range(4, 8)) for u in range(NSUB)]
                pp = prep_pre(w2T, cn, sl[1], aB, tB, False, flag)
                for r in range(7):
                    dy(NSUB - 1, r, pp[PA * r // 7:PA * (r + 1) // 7])
                put = lambda dst: lambda i, j, v: dw_put(dst, c, k == 1, DK * i, v, HF * j)
                dw_main(gS, gh, put(dw2p), flag)
                dw_main(yS.at[2 - k], gd, put(dw1p), flag)
                dw_put(dw2p, c, k == 1, 2 * DK, dw_tail(gS, 64, gh, flag, pp[PA:PB_]))
                d1 = dw_put(dw1p, c, k == 1, 2 * DK, dw_tail(yS.at[2 - k], 80, gd, flag, pp[PB_:]))
                b1s[1:2, pl.ds(pl.multiple_of(c * TF, TF), TF)] = d1[D - 2 * DK:D - 2 * DK + 1]

            @pl.when(k == 2)
            def _():
                out1(c).start()
                out2(c).start()
            return sl[1], sl[2], sl[0]
        lax.fori_loop(0, NC, body, (jnp.int32(0), jnp.int32(1), jnp.int32(2)))

    def c_io(dst, t):
        return cp(io.at[t], dst.at[0, :, tok(t)], 0)

    def bwd_a(l):
        def s1a(j, t, tie=None):
            dy = comb(ad, j, t, tie)
            st2(xs.at[t], j, dy)
            return dy, dy * ld2(yr.at[l, t], j).astype(f32)

        def s1b(j, t, z, m1, m2):
            h, o = 2 * (j // 3), R1 * (j % 3)
            base = jnp.where(l == 1, ld1(io.at[t], j).astype(f32),
                             jnp.concatenate([ax[t, h, o:o + R1, :], ax[t, h + 1, o:o + R1, :]], axis=1))
            dx = base + st[l, t, 1:2, :] * (ld1(xs.at[t], j) - m1 - ld1(yr.at[l, t], j).astype(f32) * m2)
            _st(xs.at[t], R1 * j, dx)
            _st(dxs.at[z], R1 * j, dx)
            return dx

        def body(t, z, carry):
            flag = zs[0] > 0 if OF & 4 else t < 0
            tn = nxt(t)
            pqn = lambda r0, r1: _ld(qk.at[l, t], r0, r1)
            dxb = lambda r0, r1: _ld(dxs.at[z], r0, r1)
            s1, s2, dpqn, prod = [], [], [], []
            for j in range(CH):
                d = _nn(ld1(Wp.at[l], j), dxb(0, D))
                g = s1a(j, tn, [None, d, dpqn[j - 1] if j else None][TI])
                s1.append(_csum(g[0]))
                s2.append(_csum(g[1]))
                dpqn.append(_gate(flag, d, g[1:], RA))
                prod.append((dpqn[j] * pqn(R1 * j, R1 * (j + 1)).astype(f32)).astype(bf16))

            m1, m2 = _cmean(sum(s1)), _cmean(sum(s2)) * (1.0 + LN_EPS)
            sb = lambda j: s1b(j, tn, 1 - z, m1, m2)

            def out(j):
                v = comb(ax, j, t)
                st2(io.at[t], j, v)
                return v

            def dq(j):
                R = _head_rows(lambda h: rr[l, t, h:h + 1, :], R1 * j, R1 * (j + 1))
                a = jnp.minimum(pqn(R1 * j, R1 * (j + 1)).astype(f32) - PHI_EPS * R, R)
                C = _head_rows(lambda h: c[h:h + 1], R1 * j, R1 * (j + 1))
                v = a * (dpqn[j] - C * jnp.tile(ld1(zcol.at[l], j), (1, TS // 128)))
                _st(qa.at[t], R1 * j, v)
                return v
            dWp[0:R1, 0:512] += _gate(flag, _nt(pqn(0, R1), dxb(0, 512)), [sb(0), sb(1), sb(2)], RA)
            c = _nn(_ld(hs, 0, H), jnp.concatenate(prod, axis=0))
            dxc = jnp.concatenate([dxb(512, D), *_split(c)], axis=0)
            dWp[R1:2 * R1, 0:512] += _gate(flag, _nt(pqn(R1, 2 * R1), dxb(0, 512)), [sb(3), sb(4), sb(5)], RA)
            for j, js, os_ in BV:
                if j < 0:
                    dWp[0:2 * R1, 512:640] += _gate(flag, _nt(pqn(0, 2 * R1), dxc), [dq(i) for i in js], RA)
                else:
                    dWp[R1 * j:R1 * (j + 1), :] += _gate(
                        flag, _nt(pqn(R1 * j, R1 * (j + 1)), jnp.concatenate([dxb(0, 512), dxc], axis=0)),
                        [dq(i) for i in js] + [out(i) for i in os_], RA)

            @pl.when(l == 1)
            def _():
                c_io(out_hbm, t).start()
            return carry
        p = [s1a(j, 0) for j in range(CH)]
        m1, m2 = _cmean(sum(_csum(a) for a, _ in p)), _cmean(sum(_csum(b) for _, b in p)) * (1.0 + LN_EPS)
        for j in range(CH):
            s1b(j, 0, 0, m1, m2)
        lax.fori_loop(0, NTB // 2, pair(body), 0)

    def mid_bwd(l):
        dz = -jnp.sum(jnp.where(own[...] > 0, dWp[:, 512:640], 0.0), axis=1, keepdims=True)
        zhi, zlo = _split(dz)
        lane = lax.broadcasted_iota(jnp.int32, (D, DP - D), 1)
        zc = jnp.where(lane == 0, zhi.astype(f32), jnp.where(lane == 1, zlo.astype(f32), 0.0))
        win = [(_win(g), GR * g - _win(g)) for g in range(NG)]
        dw = [dWp[w:w + GW, 0:D].astype(bf16) for w, o in win]
        dkv = [jnp.where(masks[g % 2], _nt(dw[g], wo[w:w + GW, :]), 0.0) for g, (w, o) in enumerate(win)]
        rows = [_nn(dkv[g][o:o + GR].astype(bf16), _ld(wqkvT, 2 * D + w, 2 * D + w + GW)) for g, (w, o) in enumerate(win)]
        a = jnp.concatenate(rows, axis=0)
        _st(a1, 0, jnp.concatenate([a, zc], axis=1))
        _st(wdu, 0, a.astype(bf16).T, slice(2 * D, 3 * D))
        dWp[...] = jnp.zeros_like(dWp)
        for g, (w, o) in enumerate(win):
            dwo_a[GR * g:GR * (g + 1), :] += _nn(kvT[l, g], dw[g])
        for g, (w, o) in enumerate(win):
            dwvT[GR * g:GR * (g + 1), :] += _nn(dkv[g].T[o:o + GR].astype(bf16), GT[l, w:w + GW, 0:D].astype(bf16))

    def bwd_b(l):
        def body(t, carry):
            flag = zs[0] > 0 if OF & 8 else t < 0
            Q = lambda r0, r1: jnp.concatenate(([_ld(qa.at[t], r0, min(r1, D))] if r0 < D else [])
                                               + ([_ld(qk.at[l, t], max(r0 - D, 0), r1 - D)] if r1 > D else []), axis=0)
            U = lambda r0, r1: _ld(uT.at[l, t], r0, r1)
            for j in range(CH):
                dpk = _nn(ld1(a1, j), U(0, DP))
                zero_ad(flag, dpk, j, t)
                _st(qk.at[l, t], R1 * j, dpk * jnp.minimum(ld1(qk.at[l, t], j, D).astype(f32) - PHI_EPS, 1.0))
            r = st[l, t, 0:1, :]
            s1, s2 = [], []
            for j in range(CH):
                du = sum(_nn(ld1(wdu, j, 0, slice(a, b)), Q(a, b)) for a, b in ((2 * D, 3 * D), (0, 512), (512, 2 * D)))
                if j < 5:
                    du = _gate(flag, du, beta_io(prv(t, 2), prv(t, 2) % 2, j, t < 2), 8)
                xs[t, R1 * j:R1 * (j + 1), :] += r * du
                s1.append(_csum(du))
                s2.append(_csum(du * U(R1 * j, R1 * (j + 1)).astype(f32)))
            m1, m2 = r * _cmean(sum(s1)), r * _cmean(sum(s2))
            for j in range(CH):
                dx = ld1(xs.at[t], j) - m1 - U(R1 * j, R1 * (j + 1)).astype(f32) * m2
                _st(xs.at[t], R1 * j, dx)
                _st(io.at[t], R1 * j, dx)
                h, o = 2 * (j // 3), R1 * (j % 3)
                ax[t, h, o:o + R1, :] = dx[:, 0:P]
                ax[t, h + 1, o:o + R1, :] = dx[:, P:TS]
                dwqk[R1 * j:R1 * (j + 1), :] += _gate(flag, _nt(U(R1 * j, R1 * (j + 1)), Q(0, 2 * D)), [dx], 8)

            @pl.when(l == 0)
            def _():
                c_io(dx_hbm, t).start()
            return carry
        lax.fori_loop(0, NTB, body, 0)

        @pl.when(l == 1)
        def _():
            for tq in (NTB - 2, NTB - 1):
                for i in range(5):
                    beta_io(tq, tq % 2, i)

    c_dwo = cp(wo, dwo_hbm, 2)
    wv = [stg(j, 2 * D + TF * j, min(TF, D - TF * j)) for j in range(3)]
    c_dwv = [cp(buf, dwqkv_hbm.at[:, cols], 5) for buf, cols in wv]

    def stage(k, carry):
        @pl.when(k < 2)
        def _():
            fwd_a(k)

            @pl.when(k == 0)
            def _():
                for c in c_g:
                    c.start()
                for c in [c_wo] + c_w(0):
                    c.wait()
                for c in c_w(1):
                    c.start()
            prep_t(w12.at[k], 0)
            prep_pre(None, 0, 0, aFB.at[k], None, False)
            prep_tail(w1, 0, 0, tF, True)
            prep_tail(w2T, 0, 0, tB, False)
            mid_fwd(k)
            fwd_b(k)

        @pl.when(k == 0)
        def _():
            for c in c_g:
                c.wait()
        mlp(k)

        @pl.when(k > 0)
        def _():
            l = 2 - k
            bwd_a(l)
            mid_bwd(l)

            @pl.when(k == 1)
            def _():
                for t in range(NTB):
                    c_io(out_hbm, t).wait()

            @pl.when(k == 2)
            def _():
                wo[...] = dwo_a[...].astype(bf16)
                c_dwo.start()
                for c in range(NC):
                    out1(c).wait()
                for j, (buf, _) in enumerate(wv):
                    buf[...] = dwvT[TF * j:TF * j + buf.shape[1], :].astype(bf16).T
                    c_dwv[j].start()
                ones = jnp.ones((16, 128), bf16)
                b2v[...] = sum(_nt(ones, v) for v in _split(db2a[...]))[0:1].reshape(D).astype(bf16)
                b1v[...] = b1s[1:2].reshape(F).astype(bf16)
                for c in c_db:
                    c.start()
            bwd_b(l)
        return carry
    lax.fori_loop(0, 3, stage, 0)

    c_dwq = []
    for j in range(5):
        buf, cols = stg(3 + j, TF * j, min(TF, 2 * D - TF * j))
        buf[...] = dwqk[:, cols].astype(bf16)
        c_dwq.append(cp(buf, dwqkv_hbm.at[:, cols], 1))
        c_dwq[-1].start()
    for c in c_w(1) + [c_dwo] + c_dwv + c_db:
        c.wait()
    for c in range(NC):
        out2(c).wait()
    for t in range(NTB):
        c_io(dx_hbm, t).wait()
    for c in c_dwq:
        c.wait()


@jax.jit
def pallas_interleave_layers__linear_attn_block__mixer_channel_mlp__prompt_kernel(A_x, A_wqkv, A_wo, B_x, B_w1, B_b1, B_w2, B_b2, grad_out):
    anyspec = pl.BlockSpec(memory_space=pl.ANY)
    V = pltpu.VMEM

    def PB(*s):
        return V(s[:-2] + (s[-2] // 2, s[-1]), u32) if PK else V(s, bf16)
    scratch = [
        V((NTB, D, TS), bf16),
        V((D, 64), bf16),
        PB(D, 3 * D),
        PB(3 * D, D),
        V((D, D), bf16),
        V((2, 3, D, TF), bf16),
        V((NTB + 2, D, TS), f32),
        V((NTB, 7, DM, P), f32),
        V((NTB, 7, DM, P), f32),
        PB(NTB, BT + 64, TS),
        PB(2, D, TS),
        PB(2, NTB, DP, TS),
        PB(NTB, D, TS),
        PB(2, NTB + 1, 2 * D, TS),
        PB(2, NTB, BT + 80, TS),
        PB(2, NTB, D, TS),
        PB(NC + 1, 4, NSUB, HF, SW),
        V((NC, DP, TF), bf16),
        V((NC, D, TF), bf16),
        PB(2, 25, 64, 256),
        PB(TF, 80),
        PB(TF, 64),
        PB(TF, 2 * DK),
        V((8, F), f32),
        V((2, NTB + 2, 8, TS), f32),
        V((2, NTB + 2, H, TS), f32),
        V((2, D, DP), f32),
        PB(2, D, D),
        PB(D, D),
        V((2, NG, GR, GW), bf16),
        PB(H, D),
        PB(H, D),
        V((2, D, 128), f32),
        V((D, 640), f32),
        V((D, 2 * D), f32),
        V((D, D), f32),
        V((D, D), f32),
        PB(D, DP),
        V((D, 128), f32),
        V((D, 128), f32),
        V((D, 128), f32),
        V((F + 768,), bf16),
        V((D,), bf16),
        pltpu.SMEM((1,), jnp.int32),
        pltpu.SemaphoreType.DMA((8,)),
    ]
    sds = jax.ShapeDtypeStruct
    outs = pl.pallas_call(
        _kernel,
        in_specs=[anyspec] * 8,
        out_specs=[anyspec] * 8,
        out_shape=[sds((1, D, S), bf16), sds((1, D, S), bf16), sds((D, 3 * D), bf16), sds((D, D), bf16),
                   sds((D, F), bf16), sds((F,), bf16), sds((D, F), bf16), sds((D,), bf16)],
        scratch_shapes=scratch,
        compiler_params=pltpu.CompilerParams(vmem_limit_bytes=128 * 1024 * 1024 - 128 * 1024,
                                             disable_bounds_checks=True),
    )(jnp.swapaxes(A_x, 1, 2), A_wqkv, A_wo, B_w1, B_b1, B_w2.T, B_b2,
      jnp.swapaxes(grad_out, 1, 2))
    out, dx, dwqkv, dwo, dw1, db1, dw2, db2 = outs
    return (jnp.swapaxes(out, 1, 2), jnp.swapaxes(dx, 1, 2), dwqkv, dwo, dw1, db1, dw2.T, db2)
```
